```python
import jax
import jax.numpy as jnp

def _softmax(x, axis=-1):
    return jax.nn.softmax(x, axis=axis)

def _gelu(x):
    return jax.nn.gelu(x, approximate=True)

def _silu(x):
    return jax.nn.silu(x)

def _sigmoid(x):
    return jax.nn.sigmoid(x)

def _layernorm(x, axis=-1, eps=1e-05):
    m = jnp.mean(x, axis=axis, keepdims=True)
    v = jnp.var(x, axis=axis, keepdims=True)
    return (x - m) / jnp.sqrt(v + eps)

def _scatter_add(tgt, idx, src, axis=0):
    return tgt.at[idx].add(src)

def _segment_sum(src, seg, n):
    return jax.ops.segment_sum(src, seg, n)

class _Rng:

    def __init__(self, key):
        self._k = key

    def _next(self):
        self._k, sub = jax.random.split(self._k)
        return sub

    def normal(self, shape):
        return jax.random.normal(self._next(), shape, dtype=jnp.bfloat16)

    def randint(self, lo, hi, shape):
        return jax.random.randint(self._next(), shape, lo, hi, dtype=jnp.int32)

    def uniform(self, shape, lo=0.0, hi=1.0):
        return jax.random.uniform(self._next(), shape, jnp.bfloat16, lo, hi)

    def permutation(self, n):
        return jax.random.permutation(self._next(), n)
kernel_name = 'adaLN_cond__sliding_local_dilated__glu_gated_bilinear__prompt'

def setup_inputs():
    _rng = _Rng(jax.random.key(int.from_bytes(__import__("os").urandom(4), "little")))
    _w = lambda a: (lambda t: t.astype(jnp.bfloat16) if jnp.issubdtype(t.dtype, jnp.floating) else t)(jnp.asarray(a))

    def _A_setup():
        B, S, D = (1, 2048, 576)
        return {'x': _w((lambda *s: _rng.normal(s) * 0.05)(B, S, D)), 'wqkv': _w((lambda *s: _rng.normal(s) * 0.05)(D, 3 * D)), 'wo': _w((lambda *s: _rng.normal(s) * 0.05)(D, D))}
    _A_in = _A_setup()

    def _B_setup():
        B, S, D, F = (1, 2048, 576, 4608)
        return {'x': _w((lambda *s: _rng.normal(s) * 0.05)(B, S, D)), 'w_gate': _w((lambda *s: _rng.normal(s) * 0.05)(D, F) * D ** (-0.5)), 'w_up': _w((lambda *s: _rng.normal(s) * 0.05)(D, F) * D ** (-0.5)), 'w_down': _w((lambda *s: _rng.normal(s) * 0.05)(F, D) * F ** (-0.5))}
    _B_in = _B_setup()
    return {'A_x': _A_in['x'], 'A_wqkv': _A_in['wqkv'], 'A_wo': _A_in['wo'], 'B_x': _B_in['x'], 'B_w_gate': _B_in['w_gate'], 'B_w_up': _B_in['w_up'], 'B_w_down': _B_in['w_down'], 'c': _w((lambda *s: _rng.normal(s) * 0.05)(1, 576)), 'w_mod': _w((lambda *s: _rng.normal(s) * 0.05)(576, 6 * 576) * 576 ** (-0.5))}

def reference(A_x, A_wqkv, A_wo, B_x, B_w_gate, B_w_up, B_w_down, c, w_mod):

    def _A_ref(x, wqkv, wo):
        B, S, D = x.shape
        H = 32
        Dh = D // H
        W, dil = (8, 2)
        qkv = (lambda x, *d: x.transpose(*d))((x @ wqkv).reshape(B, S, 3, H, Dh), 2, 0, 3, 1, 4)
        q, k, v = (qkv[0], qkv[1], qkv[2])
        scale = Dh ** (-0.5)
        pos = jnp.arange(S)
        off = jnp.arange(W) * dil
        idx = pos[:, None] - off[None, :]
        mask = idx >= 0
        idx_c = jnp.where(mask, idx, 0).reshape(-1)
        kg = k[:, :, idx_c, :].reshape(B, H, S, W, Dh)
        vg = v[:, :, idx_c, :].reshape(B, H, S, W, Dh)
        logits = jnp.einsum('bhsd,bhswd->bhsw', q, kg) * scale
        logits = jnp.where(mask[None, None, :, :], logits, -1000000000.0)
        attn = _softmax(logits, axis=-1)
        o = jnp.einsum('bhsw,bhswd->bhsd', attn, vg)
        return (lambda x, *d: x.transpose(*d))(o, 0, 2, 1, 3).reshape(B, S, D) @ wo

    def _B_ref(x, w_gate, w_up, w_down):
        g = jnp.einsum('bsd,df->bsf', x, w_gate)
        u = jnp.einsum('bsd,df->bsf', x, w_up)
        h = g * u
        return jnp.einsum('bsf,fd->bsd', h, w_down)
    x = A_x
    mod = (_silu(c) @ w_mod).reshape(c.shape[0], 6, 1, -1)
    sa, ca, ga, sb, cb, gb = (mod[:, 0].copy(), mod[:, 1].copy(), mod[:, 2].copy(), mod[:, 3].copy(), mod[:, 4].copy(), mod[:, 5].copy())
    h = _layernorm(x, axis=-1) * (1 + ca) + sa
    x = x + ga * _A_ref(h, A_wqkv, A_wo)
    h = _layernorm(x, axis=-1) * (1 + cb) + sb
    x = x + gb * _B_ref(h, B_w_gate, B_w_up, B_w_down)
    return x
```

```python
import functools
import jax
import jax.numpy as jnp
from jax import lax
import jax.experimental.pallas as pl
import jax.experimental.pallas.tpu as pltpu

D, H, DH, WIN, DIL, F, S = 576, 32, 18, 8, 2, 4608, 2048
EPS = 1e-5
f32, bf16 = jnp.float32, jnp.bfloat16


def _ln_mod(x, scale, shift):
    m = jnp.sum(x, axis=0, keepdims=True) * (1.0 / D)
    xc = x - m
    v = jnp.sum(xc * xc, axis=0, keepdims=True) * (1.0 / D)
    return xc * lax.rsqrt(v + EPS) * scale + shift


def kernel(xT_hbm, wqkv_hbm, wo_hbm, wg_hbm, wu_hbm, wdT_hbm, c_hbm, wmod_hbm, out_hbm,
           c_v, wmod_v, x_v, wqkv_v, wo_v, tmp_v, wqkvT_v, woT_v, modc_v,
           h_v, q_v, k_v, v_v, o_v, x1_v, h2_v, wg_v, wu_v, wd_v, wguT_v, acc_v, out_v, sems,
           *, TN, FC, HR, FN):
    NT = S // TN
    NC = F // FC
    cp = pltpu.make_async_copy
    d_c = cp(c_hbm, c_v, sems.at[0])
    d_m0 = cp(wmod_hbm.at[:, pl.ds(0, 1152)], wmod_v.at[:, pl.ds(0, 1152)], sems.at[1])
    d_qkv = cp(wqkv_hbm, wqkv_v, sems.at[2])
    d_x = cp(xT_hbm, x_v, sems.at[3])
    d_wo = cp(wo_hbm, wo_v, sems.at[4])
    d_m1 = cp(wmod_hbm.at[:, pl.ds(1152, 2304)], wmod_v.at[:, pl.ds(1152, 2304)], sems.at[5])
    d_wg = cp(wg_hbm, wg_v, sems.at[6])
    d_wu = cp(wu_hbm, wu_v, sems.at[7])
    d_wd = cp(wdT_hbm, wd_v, sems.at[8])
    d_c.start(); d_qkv.start(); d_m0.start(); d_x.start()

    d_qkv.wait()
    zpad = jnp.zeros((64, 128), f32)
    for kb in range(5):
        kw = min(128, D - 128 * kb)
        for j in range(14):
            w = min(128, 3 * D - 128 * j)
            blk = wqkv_v[pl.ds(128 * kb, kw), pl.ds(128 * j, w)].astype(f32)
            if w < 128:
                blk = jnp.concatenate([blk, jnp.zeros((kw, 128 - w), f32)], axis=1)
            if kw < 128:
                blk = jnp.concatenate([blk, zpad], axis=0)
            tmp_v[kb, pl.ds(128 * j, w), :] = blk.T[0:w]
        for p in range(3):
            for d in range(DH):
                r = tmp_v[kb, pl.ds(p * D + d, H, stride=DH), :]
                wqkvT_v[pl.ds(p * D + d * H, H), pl.ds(128 * kb, kw)] = r[:, 0:kw].astype(bf16)

    d_c.wait(); d_m0.wait()
    d_wo.start(); d_m1.start()
    cc = c_v[...].astype(f32)
    sc = jnp.broadcast_to(cc * jax.nn.sigmoid(cc), (16, D)).astype(bf16)

    def mod_cols(lo, hi):
        m = jnp.dot(sc, wmod_v[:, pl.ds(lo, hi - lo)], preferred_element_type=f32)[0:8]
        lane = lo + lax.broadcasted_iota(jnp.int32, m.shape, 1)
        one = ((lane >= D) & (lane < 2 * D)) | ((lane >= 4 * D) & (lane < 5 * D))
        m = m + jnp.where(one, 1.0, 0.0)
        for j in range((hi - lo) // 128):
            blk = jnp.tile(m[:, 128 * j:128 * (j + 1)], (16, 1))
            modc_v[pl.ds(lo + 128 * j, 128), :] = blk.T
    mod_cols(0, 1152)
    d_x.wait()

    def col(ref, j):
        return ref[:, pl.ds(128 * j, 128)]

    def ln1(t):
        for j in range(t * TN // 128, (t + 1) * TN // 128):
            h = _ln_mod(col(x_v, j).astype(f32), modc_v[pl.ds(D, D), :], modc_v[pl.ds(0, D), :])
            h_v[:, pl.ds(128 * j, 128)] = h.astype(bf16)

    def qkv(t):
        h = h_v[:, pl.ds(t * TN, TN)]
        q_v[:, pl.ds(t * TN, TN)] = jnp.dot(wqkvT_v[pl.ds(0, D), :], h, preferred_element_type=f32)
        k_v[:, pl.ds(128 + t * TN, TN)] = jnp.dot(wqkvT_v[pl.ds(D, D), :], h, preferred_element_type=f32)
        v_v[:, pl.ds(128 + t * TN, TN)] = jnp.dot(wqkvT_v[pl.ds(2 * D, D), :], h, preferred_element_type=f32)
        if t == 0:
            k_v[:, pl.ds(0, 128)] = jnp.broadcast_to(k_v[:, pl.ds(128, 1)], (D, 128))
            v_v[:, pl.ds(0, 128)] = jnp.broadcast_to(v_v[:, pl.ds(128, 1)], (D, 128))

    lane = lax.broadcasted_iota(jnp.int32, (HR, 128), 1)
    scale = DH ** -0.5

    def shifted(ref, r, j):
        cur = ref[pl.ds(r, HR), pl.ds(128 * (j + 1), 128)]
        prev = ref[pl.ds(r, HR), pl.ds(128 * j, 128)]
        out = [cur]
        for w in range(1, WIN):
            out.append(pltpu.roll(jnp.where(lane < 128 - DIL * w, cur, prev), DIL * w, 1))
        return out

    def attn(t):
        for j in range(t * TN // 128, (t + 1) * TN // 128):
            for hg in range(H // HR):
                lg = [None] * WIN
                for d in range(DH):
                    r = d * H + hg * HR
                    q = q_v[pl.ds(r, HR), pl.ds(128 * j, 128)]
                    ks = shifted(k_v, r, j)
                    for w in range(WIN):
                        lg[w] = q * ks[w] if d == 0 else lg[w] + q * ks[w]
                lg = [l * scale for l in lg]
                if j == 0:
                    lg = [l if w == 0 else jnp.where(lane >= DIL * w, l, -1e9) for w, l in enumerate(lg)]
                mx = functools.reduce(jnp.maximum, lg)
                e = [jnp.exp(l - mx) for l in lg]
                inv = 1.0 / functools.reduce(lambda a, b: a + b, e)
                p = [x * inv for x in e]
                for d in range(DH):
                    r = d * H + hg * HR
                    vs = shifted(v_v, r, j)
                    o = p[0] * vs[0]
                    for w in range(1, WIN):
                        o = o + p[w] * vs[w]
                    o_v[pl.ds(r, HR), pl.ds(128 * j, 128)] = o.astype(bf16)

    def wo_ln2(t):
        y = jnp.dot(woT_v[...], o_v[:, pl.ds(t * TN, TN)], preferred_element_type=f32)
        for jj in range(TN // 128):
            j = t * TN // 128 + jj
            x1 = col(x_v, j).astype(f32) + modc_v[pl.ds(2 * D, D), :] * y[:, 128 * jj:128 * (jj + 1)]
            x1_v[:, pl.ds(128 * j, 128)] = x1
            h2 = _ln_mod(x1, modc_v[pl.ds(4 * D, D), :], modc_v[pl.ds(3 * D, D), :])
            h2_v[:, pl.ds(128 * j, 128)] = h2.astype(bf16)

    ln1(0)
    qkv(0)
    d_wo.wait(); d_m1.wait()
    d_wg.start(); d_wu.start(); d_wd.start()
    mod_cols(1152, 3456)
    for nb in range(5):
        nw = min(128, D - 128 * nb)
        blk = wo_v[:, pl.ds(128 * nb, nw)].astype(f32)
        if nw < 128:
            blk = jnp.concatenate([blk, jnp.zeros((D, 128 - nw), f32)], axis=1)
        tmp_v[nb, pl.ds(0, D), :] = blk
        for eb in range(5):
            ds_ = range(4 * eb, min(4 * eb + 4, DH))
            rows = [tmp_v[nb, pl.ds(d, H, stride=DH), :] for d in ds_]
            ew = H * len(rows)
            if ew < 128:
                rows.append(zpad)
            woT_v[pl.ds(128 * nb, nw), pl.ds(128 * eb, ew)] = jnp.concatenate(rows, axis=0).T[0:nw, 0:ew].astype(bf16)
    for t in range(NT):
        if t + 1 < NT:
            ln1(t + 1)
            qkv(t + 1)
        attn(t)
        if t > 0:
            wo_ln2(t - 1)
    wo_ln2(NT - 1)

    d_wg.wait(); d_wu.wait(); d_wd.wait()

    def prep(j, slot):
        off = pl.multiple_of(j * FC, FC)
        wguT_v[slot, pl.ds(0, FC), :] = wg_v[:, pl.ds(off, FC)].T
        wguT_v[slot, pl.ds(FC, FC), :] = wu_v[:, pl.ds(off, FC)].T

    def ffn(j, slot, first, last):
        off = pl.multiple_of(j * FC, FC)
        for t in range(S // FN):
            sl = pl.ds(t * FN, FN)
            h = h2_v[:, sl]
            g = jnp.dot(wguT_v[slot, pl.ds(0, FC), :], h, preferred_element_type=f32)
            u = jnp.dot(wguT_v[slot, pl.ds(FC, FC), :], h, preferred_element_type=f32)
            y = jnp.dot(wd_v[:, pl.ds(off, FC)], (g * u).astype(bf16), preferred_element_type=f32)
            if not first:
                y = y + acc_v[:, sl]
            if not last:
                acc_v[:, sl] = y
            else:
                for jj in range(FN // 128):
                    c = pl.ds(t * FN + 128 * jj, 128)
                    out_v[:, c] = (x1_v[:, c] + modc_v[pl.ds(5 * D, D), :] * y[:, 128 * jj:128 * (jj + 1)]).astype(bf16)
                cp(out_v.at[:, sl], out_hbm.at[:, sl], sems.at[9 + t]).start()

    prep(0, 0)
    prep(1, 1)
    ffn(0, 0, True, False)

    def body(j, _):
        slot = j % 2
        prep(j + 1, 1 - slot)
        ffn(j, slot, False, False)
        return _
    lax.fori_loop(1, NC - 1, body, None)
    ffn(NC - 1, (NC - 1) % 2, False, True)
    for t in range(S // FN):
        sl = pl.ds(t * FN, FN)
        cp(out_v.at[:, sl], out_hbm.at[:, sl], sems.at[9 + t]).wait()


def make(TN=256, FC=512, HR=16, FN=256):
    @jax.jit
    def f(A_x, A_wqkv, A_wo, B_x, B_w_gate, B_w_up, B_w_down, c, w_mod):
        xT = A_x[0].T
        wdT = B_w_down.T
        hbm = pl.BlockSpec(memory_space=pltpu.HBM)
        V = pltpu.VMEM
        outT = pl.pallas_call(
            functools.partial(kernel, TN=TN, FC=FC, HR=HR, FN=FN),
            in_specs=[hbm] * 8,
            out_specs=hbm,
            out_shape=jax.ShapeDtypeStruct((D, S), bf16),
            scratch_shapes=[
                V((1, D), bf16), V((D, 6 * D), bf16), V((D, S), bf16), V((D, 3 * D), bf16), V((D, D), bf16),
                V((5, 3 * D, 128), f32), V((3 * D, D), bf16), V((D, D), bf16), V((6 * D, 128), f32),
                V((D, S), bf16), V((D, S), f32), V((D, S + 128), f32), V((D, S + 128), f32), V((D, S), bf16),
                V((D, S), f32), V((D, S), bf16), V((D, F), bf16), V((D, F), bf16), V((D, F), bf16),
                V((2, 2 * FC, D), bf16), V((D, S), f32), V((D, S), bf16),
                pltpu.SemaphoreType.DMA((9 + S // FN,)),
            ],
            compiler_params=pltpu.CompilerParams(vmem_limit_bytes=120 * 1024 * 1024),
        )(xT, A_wqkv, A_wo, B_w_gate, B_w_up, wdT, c, w_mod)
        return outT.T[None]
    return f


pallas_adaLN_cond__sliding_local_dilated__glu_gated_bilinear__prompt_kernel = make()
```

```python
import functools
import jax
import jax.numpy as jnp
from jax import lax
import jax.experimental.pallas as pl
import jax.experimental.pallas.tpu as pltpu

D, H, DH, WIN, DIL, F, S = 576, 32, 18, 8, 2, 4608, 2048
EPS = 1e-5
f32, bf16, u32 = jnp.float32, jnp.bfloat16, jnp.uint32
TN = 256
NT = S // TN


def _dot(a, b):
    return jnp.dot(a, b, preferred_element_type=f32)


def _to_words(x):
    return pltpu.bitcast(x.astype(bf16), u32)


def _from_words(x):
    return pltpu.bitcast(x, bf16)


def _halves(x):
    return tuple(pltpu.unpack_elementwise(x, index=i, packed_dtype=bf16, unpacked_dtype=f32) for i in range(2))


def _comb_a(a11, a12, a21, a22):
    return [a11 + a22, a21 + a22, a11, a22, a11 + a12, a21 - a11, a12 - a22]


def _comb_b(b11, b12, b21, b22):
    return [b11 + b22, b11, b12 - b22, b21 - b11, b22, b11 + b12, b21 + b22]


def _comb_c(m):
    return (m[0] + m[3] - m[4] + m[6], m[2] + m[4], m[1] + m[3], m[0] - m[1] + m[2] + m[5])


def _ln_mod(x, scale, shift):
    m = jnp.sum(x, axis=0, keepdims=True) * (1.0 / D)
    xc = x - m
    v = jnp.sum(xc * xc, axis=0, keepdims=True) * (1.0 / D)
    return xc * lax.rsqrt(v + EPS) * scale + shift


def kernel(xT_hbm, wqkv_hbm, wo_hbm, wg_hbm, wu_hbm, wdT_hbm, c_hbm, wmod_hbm, out_hbm,
           c_v, wmod_v, x_v, wqkv_v, wo_v, tmp_v, wqkvT_v, woT_v, modc_v,
           h_v, q_v, k_v, v_v, o_v, x1_v, hb_v, hr_v, wg_v, wu_v, wd_v, a_v, ar_v, ad_v, g_v, acc_v, out_v, sems,
           *, FC, FT, scopes):
    NC = F // FC
    HC = FC // 2
    cp = pltpu.make_async_copy
    scope = jax.named_scope if scopes else (lambda name: __import__('contextlib').nullcontext())
    sem_i = iter(range(64))
    d_c = cp(c_hbm, c_v, sems.at[next(sem_i)])

    def colcp(src, dst, lo, hi):
        return cp(src.at[:, pl.ds(lo, hi - lo)], dst.at[:, pl.ds(lo, hi - lo)], sems.at[next(sem_i)])
    d_m0 = colcp(wmod_hbm, wmod_v, 0, 1152)
    d_m1 = colcp(wmod_hbm, wmod_v, 1152, 3456)
    d_x0 = colcp(xT_hbm, x_v, 0, 2 * TN)
    d_x1 = colcp(xT_hbm, x_v, 2 * TN, S)
    d_qkv = [colcp(wqkv_hbm, wqkv_v, lo, hi) for lo, hi in ((0, 640), (640, 1152), (1152, 1728))]
    d_wo = cp(wo_hbm, wo_v, sems.at[next(sem_i)])
    d_f0 = [colcp(s, d, 0, 2 * FC) for s, d in ((wg_hbm, wg_v), (wu_hbm, wu_v), (wdT_hbm, wd_v))]
    d_f1 = [colcp(s, d, 2 * FC, F) for s, d in ((wg_hbm, wg_v), (wu_hbm, wu_v), (wdT_hbm, wd_v))]
    out_sem0 = next(sem_i)

    d_c.start(); d_m0.start(); d_x0.start(); d_qkv[0].start()

    with scope('w_m0'):
        d_c.wait(); d_m0.wait()
    d_qkv[1].start()
    cc = c_v[...].astype(f32)
    sc = jnp.broadcast_to(cc * jax.nn.sigmoid(cc), (16, D)).astype(bf16)

    def mod_cols(lo, hi):
        m = _dot(sc, wmod_v[:, pl.ds(lo, hi - lo)])[0:8]
        lane = lo + lax.broadcasted_iota(jnp.int32, m.shape, 1)
        one = ((lane >= D) & (lane < 2 * D)) | ((lane >= 4 * D) & (lane < 5 * D))
        m = m + jnp.where(one, 1.0, 0.0)
        for j in range((hi - lo) // 128):
            blk = jnp.tile(m[:, 128 * j:128 * (j + 1)], (16, 1))
            modc_v[pl.ds(lo + 128 * j, 128), :] = blk.T
    mod_cols(0, 1152)

    def mod(i):
        return modc_v[pl.ds(i * D, D), :]

    def ln1(t):
        for j in range(2 * t, 2 * t + 2):
            c = pl.ds(128 * j, 128)
            h_v[:, c] = _to_words(_ln_mod(x_v[:, c].astype(f32), mod(1), mod(0)))

    zpad = jnp.zeros((64, 128), f32)

    def prep_qkv(p):
        for kb in range(5):
            kw = min(128, D - 128 * kb)
            for j in ((0, 1, 2, 3, 4), (5, 6, 7, 8), (9, 10, 11, 12, 13))[p]:
                w = min(128, 3 * D - 128 * j)
                blk = wqkv_v[pl.ds(128 * kb, kw), pl.ds(128 * j, w)].astype(f32)
                if w < 128:
                    blk = jnp.concatenate([blk, jnp.zeros((kw, 128 - w), f32)], axis=1)
                if kw < 128:
                    blk = jnp.concatenate([blk, zpad], axis=0)
                tmp_v[kb, pl.ds(128 * j, w), :] = blk.T[0:w]
            for d in range(DH):
                r = tmp_v[kb, pl.ds(p * D + d, H, stride=DH), :]
                wqkvT_v[pl.ds((p * D + d * H) // 2, H // 2), pl.ds(128 * kb, 128)] = _to_words(r)

    def proj(p, t):
        w = _from_words(wqkvT_v[pl.ds(p * D // 2, D // 2), :])[:, 0:D]
        y = _to_words(_dot(w, _from_words(h_v[:, pl.ds(t * TN, TN)])))
        if p == 0:
            q_v[:, pl.ds(t * TN, TN)] = y
        else:
            ref = (k_v, v_v)[p - 1]
            ref[:, pl.ds(128 + t * TN, TN)] = y
            if t == 0:
                ref[:, pl.ds(0, 128)] = jnp.broadcast_to(y[:, 0:1], (D // 2, 128))

    lane = lax.broadcasted_iota(jnp.int32, (8, 128), 1)
    scale = DH ** -0.5

    def window(ref, r, j):
        cur = ref[pl.ds(r, 8), pl.ds(128 * (j + 1), 128)]
        prev = ref[pl.ds(r, 8), pl.ds(128 * j, 128)]
        yield _halves(cur)
        for w in range(1, WIN):
            yield _halves(pltpu.roll(jnp.where(lane < 128 - DIL * w, cur, prev), DIL * w, 1))

    def attn(t):
        for j in range(2 * t, 2 * t + 2):
            c = pl.ds(128 * j, 128)
            for hg in range(2):
                lg = [[None] * WIN, [None] * WIN]
                for d in range(DH):
                    r = d * (H // 2) + hg * 8
                    q = _halves(q_v[pl.ds(r, 8), c])
                    for w, k in enumerate(window(k_v, r, j)):
                        for s in range(2):
                            pr = q[s] * k[s]
                            lg[s][w] = pr if d == 0 else lg[s][w] + pr
                p = []
                for s in range(2):
                    l = [x * scale for x in lg[s]]
                    if j == 0:
                        l = [x if w == 0 else jnp.where(lane >= DIL * w, x, -1e9) for w, x in enumerate(l)]
                    mx = functools.reduce(jnp.maximum, l)
                    e = [jnp.exp(x - mx) for x in l]
                    inv = 1.0 / functools.reduce(lambda a, b: a + b, e)
                    p.append([x * inv for x in e])
                for d in range(DH):
                    r = d * (H // 2) + hg * 8
                    o = [None, None]
                    for w, v in enumerate(window(v_v, r, j)):
                        for s in range(2):
                            pr = p[s][w] * v[s]
                            o[s] = pr if w == 0 else o[s] + pr
                    o_v[pl.ds(r, 8), c] = pltpu.pack_elementwise(o, packed_dtype=bf16)

    def wo(t):
        y = _dot(_from_words(woT_v[...])[:, 0:D], _from_words(o_v[:, pl.ds(t * TN, TN)]))
        for s in range(2):
            c = pl.ds(t * TN + 128 * s, 128)
            x1_v[:, c] = x_v[:, c].astype(f32) + mod(2) * y[:, 128 * s:128 * (s + 1)]

    def ln2(t):
        h2 = [_ln_mod(x1_v[:, pl.ds(t * TN + 128 * s, 128)], mod(4), mod(3)) for s in range(2)]
        c = pl.ds(128 * t, 128)
        for i, b in enumerate(_comb_b(h2[0][0:256], h2[1][0:256], h2[0][256:512], h2[1][256:512])):
            hb_v[i, :, c] = _to_words(b)
        for s in range(2):
            hr_v[s, :, c] = _to_words(h2[s][512:576])

    def prep_wo():
        for nb in range(5):
            nw = min(128, D - 128 * nb)
            blk = wo_v[:, pl.ds(128 * nb, nw)].astype(f32)
            if nw < 128:
                blk = jnp.concatenate([blk, jnp.zeros((D, 128 - nw), f32)], axis=1)
            tmp_v[nb, pl.ds(0, D), :] = blk
            for eb in range(5):
                rows = [tmp_v[nb, pl.ds(d, H, stride=DH), :] for d in range(4 * eb, min(4 * eb + 4, DH))]
                if len(rows) < 4:
                    rows.append(zpad)
                woT_v[pl.ds(64 * nb, nw // 2), pl.ds(128 * eb, 128)] = _to_words(jnp.concatenate(rows, axis=0).T[0:nw])

    def prep_gu(j, slot, m):
        off = j * FC if isinstance(j, int) else pl.multiple_of(j * FC, FC)
        wt = (wg_v, wu_v)[m][:, pl.ds(off, FC)].T
        x = wt[:, 0:512].astype(f32)
        for i, a in enumerate(_comb_a(x[0:HC, 0:256], x[0:HC, 256:512], x[HC:FC, 0:256], x[HC:FC, 256:512])):
            a_v[slot, i, pl.ds(m * HC // 2, HC // 2), :] = _to_words(a)
        for s in range(2):
            ar_v[slot, pl.ds((2 * s + m) * HC // 2, HC // 2), :] = pltpu.bitcast(wt[s * HC:(s + 1) * HC, 512:576], u32)

    def prep_dn(j, slot):
        off = j * FC if isinstance(j, int) else pl.multiple_of(j * FC, FC)
        x = wd_v[:, pl.ds(off, FC)].astype(f32)
        for i, a in enumerate(_comb_a(x[0:288, 0:HC], x[0:288, HC:FC], x[288:576, 0:HC], x[288:576, HC:FC])):
            ad_v[slot, i] = _to_words(a)

    HN = FT * 128

    def out_copy(t):
        sl = pl.ds(t * 2 * HN, 2 * HN)
        return cp(out_v.at[:, sl], out_hbm.at[:, sl], sems.at[out_sem0 + t])

    def gate_up(slot, t):
        sl = pl.ds(t * HN, HN)
        m = [_dot(_from_words(a_v[slot, i]), _from_words(hb_v[i, :, sl])) for i in range(7)]
        ar = _from_words(ar_v[slot])
        r = [_dot(ar, _from_words(hr_v[s, :, sl])) for s in range(2)]
        c11, c12, c21, c22 = _comb_c(m)
        cs = (c11 + r[0][0:FC], c12 + r[1][0:FC], c21 + r[0][FC:2 * FC], c22 + r[1][FC:2 * FC])
        for i, b in enumerate(_comb_b(*[c[0:HC] * c[HC:FC] for c in cs])):
            g_v[t % 2, i] = _to_words(b)

    def down(slot, t, first, last):
        sl = pl.ds(t * HN, HN)
        y = [_dot(_from_words(ad_v[slot, i]), _from_words(g_v[t % 2, i])) for i in range(7)]
        if not first:
            y = [y[i] + acc_v[i, :, sl] for i in range(7)]
        if not last:
            for i in range(7):
                acc_v[i, :, sl] = y[i]
            return
        cs = _comb_c(y)
        for rh in range(2):
            rows = pl.ds(288 * rh, 288)
            for s in range(2):
                for tt in range(FT):
                    c = pl.ds((t * FT + tt) * TN + 128 * s, 128)
                    z = cs[2 * rh + s][:, 128 * tt:128 * (tt + 1)]
                    out_v[rows, c] = (x1_v[rows, c] + modc_v[pl.ds(5 * D + 288 * rh, 288), :] * z).astype(bf16)
        out_copy(t).start()

    with scope('w_x0'):
        d_x0.wait()
    d_qkv[2].start()
    ln1(0)
    with scope('w_q'):
        d_qkv[0].wait()
    d_x1.start()
    prep_qkv(0)
    ln1(1)
    proj(0, 0)
    with scope('w_k'):
        d_qkv[1].wait()
    d_wo.start(); d_m1.start()
    prep_qkv(1)
    proj(0, 1)
    with scope('w_v'):
        d_qkv[2].wait()
    prep_qkv(2)
    proj(1, 0)
    proj(2, 0)
    proj(1, 1)
    proj(2, 1)
    attn(0)
    with scope('w_rest'):
        d_x1.wait(); d_wo.wait(); d_m1.wait()
    for d in d_f0 + d_f1:
        d.start()
    ln1(2)
    mod_cols(1152, 3456)
    prep_wo()
    NFT = NT // FT
    for t in range(1, NT):
        if t + 1 < NT:
            for p in range(3):
                proj(p, t + 1)
        else:
            gate_up(0, 0)
        wo(t - 1)
        if t + 2 < NT:
            ln1(t + 2)
        attn(t)
        ln2(t - 1)
        if t == NT - 4:
            with scope('w_f0'):
                for d in d_f0:
                    d.wait()
            prep_gu(0, 0, 0)
        if t == NT - 3:
            prep_gu(0, 0, 1)
        if t == NT - 2:
            prep_dn(0, 0)
    gate_up(0, 1)
    wo(NT - 1)
    down(0, 0, True, False)
    ln2(NT - 1)

    prep_gu(1, 1, 0)
    for t in range(1, NFT):
        if t + 1 < NFT:
            gate_up(0, t + 1)
        else:
            gate_up(1, 0)
        down(0, t, True, False)
        if t == 1:
            prep_gu(1, 1, 1)
        if t == 2:
            prep_dn(1, 1)
    with scope('w_f1'):
        for d in d_f1:
            d.wait()

    def body(j, carry):
        slot = j % 2
        for t in range(NFT):
            if t + 1 < NFT:
                gate_up(slot, t + 1)
            else:
                gate_up(1 - slot, 0)
            down(slot, t, False, False)
            if t < 2:
                prep_gu(j + 1, 1 - slot, t)
            if t == 2:
                prep_dn(j + 1, 1 - slot)
        return carry
    with scope('loop'):
        lax.fori_loop(1, NC - 1, body, None)
    slot = (NC - 1) % 2
    for t in range(NFT):
        if t + 1 < NFT:
            gate_up(slot, t + 1)
        down(slot, t, False, True)
    with scope('w_out'):
        for t in range(NFT):
            out_copy(t).wait()


def make(FC=512, FT=2, scopes=False):
    @jax.jit
    def f(A_x, A_wqkv, A_wo, B_x, B_w_gate, B_w_up, B_w_down, c, w_mod):
        xT = A_x[0].T
        wdT = B_w_down.T
        hbm = pl.BlockSpec(memory_space=pltpu.HBM)
        V = pltpu.VMEM
        outT = pl.pallas_call(
            functools.partial(kernel, FC=FC, FT=FT, scopes=scopes),
            in_specs=[hbm] * 8,
            out_specs=hbm,
            out_shape=jax.ShapeDtypeStruct((D, S), bf16),
            scratch_shapes=[
                V((1, D), bf16), V((D, 6 * D), bf16), V((D, S), bf16), V((D, 3 * D), bf16), V((D, D), bf16),
                V((5, 3 * D, 128), f32), V((3 * D // 2, 640), u32), V((D // 2, 640), u32), V((6 * D, 128), f32),
                V((D // 2, S), u32), V((D // 2, S), u32), V((D // 2, S + 128), u32), V((D // 2, S + 128), u32),
                V((D // 2, S), u32), V((D, S), f32), V((7, 128, S // 2), u32), V((2, 32, S // 2), u32),
                V((D, F), bf16), V((D, F), bf16), V((D, F), bf16),
                V((2, 7, FC // 2, 256), u32), V((2, FC, 64), u32), V((2, 7, 144, FC // 2), u32), V((2, 7, FC // 4, FT * 128), u32),
                V((7, 288, S // 2), f32), V((D, S), bf16),
                pltpu.SemaphoreType.DMA((32,)),
            ],
            compiler_params=pltpu.CompilerParams(vmem_limit_bytes=120 * 1024 * 1024),
        )(xT, A_wqkv, A_wo, B_w_gate, B_w_up, wdT, c, w_mod)
        return outT.T[None]
    return f


pallas_adaLN_cond__sliding_local_dilated__glu_gated_bilinear__prompt_kernel = make()
```

```python
import contextlib
import functools
import jax
import jax.numpy as jnp
from jax import lax
import jax.experimental.pallas as pl
import jax.experimental.pallas.tpu as pltpu

D, H, DH, WIN, DIL, F, S = 576, 32, 18, 8, 2, 4608, 2048
EPS = 1e-5
f32, bf16, u32 = jnp.float32, jnp.bfloat16, jnp.uint32
TN = 256
NT = S // TN
FC = 512
NC = F // FC


def _dot(a, b):
    return jnp.dot(a, b, preferred_element_type=f32)


def _to_words(x):
    return pltpu.bitcast(x.astype(bf16), u32)


def _from_words(x):
    return pltpu.bitcast(x, bf16)


def _halves(x):
    return tuple(pltpu.unpack_elementwise(x, index=i, packed_dtype=bf16, unpacked_dtype=f32) for i in range(2))


def _add(x, y):
    return [[a + b for a, b in zip(r, s)] for r, s in zip(x, y)]


def _sub(x, y):
    return [[a - b for a, b in zip(r, s)] for r, s in zip(x, y)]


def _quad(x):
    h = len(x) // 2
    return [r[:h] for r in x[:h]], [r[h:] for r in x[:h]], [r[:h] for r in x[h:]], [r[h:] for r in x[h:]]


def _lhs_terms(x):
    if len(x) == 1:
        return [x[0][0]]
    a11, a12, a21, a22 = _quad(x)
    terms = (_add(a11, a22), _add(a21, a22), a11, a22, _add(a11, a12), _sub(a21, a11), _sub(a12, a22))
    return [z for y in terms for z in _lhs_terms(y)]


def _rhs_terms(x):
    if len(x) == 1:
        return [x[0][0]]
    b11, b12, b21, b22 = _quad(x)
    terms = (_add(b11, b22), b11, _sub(b12, b22), _sub(b21, b11), b22, _add(b11, b12), _add(b21, b22))
    return [z for y in terms for z in _rhs_terms(y)]


def _assemble(m):
    if len(m) == 1:
        return [[m[0]]]
    n = len(m) // 7
    p = [_assemble(m[i * n:(i + 1) * n]) for i in range(7)]
    c11 = _add(_sub(_add(p[0], p[3]), p[4]), p[6])
    c12 = _add(p[2], p[4])
    c21 = _add(p[1], p[3])
    c22 = _add(_add(_sub(p[0], p[1]), p[2]), p[5])
    return [a + b for a, b in zip(c11, c12)] + [a + b for a, b in zip(c21, c22)]


def _ln_mod(x, scale, shift):
    m = jnp.sum(x, axis=0, keepdims=True) * (1.0 / D)
    xc = x - m
    v = jnp.sum(xc * xc, axis=0, keepdims=True) * (1.0 / D)
    return xc * lax.rsqrt(v + EPS) * scale + shift


def kernel(xT_hbm, wqkv_hbm, wo_hbm, wg_hbm, wu_hbm, wdT_hbm, c_hbm, wmod_hbm, out_hbm,
           c_v, wmod_v, x_v, wqkv_v, wo_v, tmp_v, wqkvT_v, woT_v, modc_v,
           h_v, q_v, k_v, v_v, o_v, x1_v, hb_v, hr_v, wg_v, wu_v, wd_v, a_v, ar_v, ad_v, g_v, acc_v, out_v,
           sems, bar_sem, *, L, LD, NP, scopes, ORDER):
    n, nm, nd, nmd = 2 ** L, 7 ** L, 2 ** LD, 7 ** LD
    QC, KB, RD, KD = FC // n, 512 // n, D // nd, FC // nd
    W = 512 // n
    NFT = S // (n * W)
    WD = W * n // nd
    RP = QC // NP
    cp = pltpu.make_async_copy
    scope = jax.named_scope if scopes else (lambda name: contextlib.nullcontext())
    sem_i = iter(range(64))

    def colcp(src, dst, lo, hi):
        return cp(src.at[:, pl.ds(lo, hi - lo)], dst.at[:, pl.ds(lo, hi - lo)], sems.at[next(sem_i)])

    def make_copies(name):
        if name[0] == 'x':
            return [colcp(xT_hbm, x_v, int(name[1]) * TN, (int(name[2]) + 1) * TN)]
        if name[0] == 'f':
            return [colcp(s, d, int(name[1]) * FC, (int(name[2]) + 1) * FC)
                    for s, d in ((wg_hbm, wg_v), (wu_hbm, wu_v), (wdT_hbm, wd_v))]
        if name == 'c':
            return [cp(c_hbm, c_v, sems.at[next(sem_i)])]
        if name == 'wo':
            return [cp(wo_hbm, wo_v, sems.at[next(sem_i)])]
        if name[0] == 'm':
            return [colcp(wmod_hbm, wmod_v, *((0, 1152), (1152, 3456))[int(name[1])])]
        return [colcp(wqkv_hbm, wqkv_v, *{'q': (0, 640), 'k': (640, 1152), 'v': (1152, 1728)}[name])]

    def mod_cols(lo, hi):
        cc = c_v[...].astype(f32)
        sc = jnp.broadcast_to(cc * jax.nn.sigmoid(cc), (16, D)).astype(bf16)
        m = _dot(sc, wmod_v[:, pl.ds(lo, hi - lo)])[0:8]
        lane = lo + lax.broadcasted_iota(jnp.int32, m.shape, 1)
        one = ((lane >= D) & (lane < 2 * D)) | ((lane >= 4 * D) & (lane < 5 * D))
        m = m + jnp.where(one, 1.0, 0.0)
        for j in range((hi - lo) // 128):
            blk = jnp.tile(m[:, 128 * j:128 * (j + 1)], (16, 1))
            modc_v[pl.ds(lo + 128 * j, 128), :] = blk.T

    def mod(i):
        return modc_v[pl.ds(i * D, D), :]

    def ln1(t):
        for j in range(2 * t, 2 * t + 2):
            c = pl.ds(128 * j, 128)
            h_v[:, c] = _to_words(_ln_mod(x_v[:, c].astype(f32), mod(1), mod(0)))

    zpad = jnp.zeros((64, 128), f32)

    def prep_qkv(p):
        for kb in range(5):
            kw = min(128, D - 128 * kb)
            for j in ((0, 1, 2, 3, 4), (5, 6, 7, 8), (9, 10, 11, 12, 13))[p]:
                w = min(128, 3 * D - 128 * j)
                blk = wqkv_v[pl.ds(128 * kb, kw), pl.ds(128 * j, w)].astype(f32)
                if w < 128:
                    blk = jnp.concatenate([blk, jnp.zeros((kw, 128 - w), f32)], axis=1)
                if kw < 128:
                    blk = jnp.concatenate([blk, zpad], axis=0)
                tmp_v[kb, pl.ds(128 * j, w), :] = blk.T[0:w]
            for d in range(DH):
                r = tmp_v[kb, pl.ds(p * D + d, H, stride=DH), :]
                wqkvT_v[pl.ds((p * D + d * H) // 2, H // 2), pl.ds(128 * kb, 128)] = _to_words(r)

    def proj(p, t):
        w = _from_words(wqkvT_v[pl.ds(p * D // 2, D // 2), :])[:, 0:D]
        y = _to_words(_dot(w, _from_words(h_v[:, pl.ds(t * TN, TN)])))
        if p == 0:
            q_v[:, pl.ds(t * TN, TN)] = y
        else:
            ref = (k_v, v_v)[p - 1]
            ref[:, pl.ds(128 + t * TN, TN)] = y
            if t == 0:
                ref[:, pl.ds(0, 128)] = jnp.broadcast_to(y[:, 0:1], (D // 2, 128))

    lane = lax.broadcasted_iota(jnp.int32, (8, 128), 1)
    scale = DH ** -0.5

    def window(ref, r, j):
        cur = ref[pl.ds(r, 8), pl.ds(128 * (j + 1), 128)]
        prev = ref[pl.ds(r, 8), pl.ds(128 * j, 128)]
        yield _halves(cur)
        for w in range(1, WIN):
            yield _halves(pltpu.roll(jnp.where(lane < 128 - DIL * w, cur, prev), DIL * w, 1))

    def attn_col(j):
        c = pl.ds(128 * j, 128)
        for hg in range(2):
            lg = [[None] * WIN, [None] * WIN]
            for d in range(DH):
                r = d * (H // 2) + hg * 8
                q = _halves(q_v[pl.ds(r, 8), c])
                for w, k in enumerate(window(k_v, r, j)):
                    for s in range(2):
                        pr = q[s] * k[s]
                        lg[s][w] = pr if d == 0 else lg[s][w] + pr
            p = []
            for s in range(2):
                l = [x * scale for x in lg[s]]
                if j == 0:
                    l = [x if w == 0 else jnp.where(lane >= DIL * w, x, -1e9) for w, x in enumerate(l)]
                mx = functools.reduce(jnp.maximum, l)
                e = [jnp.exp(x - mx) for x in l]
                inv = 1.0 / functools.reduce(lambda a, b: a + b, e)
                p.append([x * inv for x in e])
            for d in range(DH):
                r = d * (H // 2) + hg * 8
                o = [None, None]
                for w, v in enumerate(window(v_v, r, j)):
                    for s in range(2):
                        pr = p[s][w] * v[s]
                        o[s] = pr if w == 0 else o[s] + pr
                o_v[pl.ds(r, 8), c] = pltpu.pack_elementwise(o, packed_dtype=bf16)

    def wo(t):
        y = _dot(_from_words(woT_v[...])[:, 0:D], _from_words(o_v[:, pl.ds(t * TN, TN)]))
        for s in range(2):
            c = pl.ds(t * TN + 128 * s, 128)
            x1_v[:, c] = x_v[:, c].astype(f32) + mod(2) * y[:, 128 * s:128 * (s + 1)]

    def term(i, per, width, r0, nr, c0=0, nc=None):
        k = 2 if width == 128 else 1
        return pl.ds((i // k) * per + r0, nr), pl.ds((i % k) * width + c0, width if nc is None else nc)

    def ln2(u):
        h2 = [_ln_mod(x1_v[:, pl.ds(128 * (n * u + s), 128)], mod(4), mod(3)) for s in range(n)]
        c = pl.ds(128 * u, 128)
        for i, b in enumerate(_rhs_terms([[h2[s][KB * k:KB * (k + 1)] for s in range(n)] for k in range(n)])):
            hb_v[pl.ds(i * KB // 2, KB // 2), c] = _to_words(b)
        for s in range(n):
            hr_v[pl.ds(32 * s, 32), c] = _to_words(h2[s][512:576])

    def prep_wo():
        for nb in range(5):
            nw = min(128, D - 128 * nb)
            blk = wo_v[:, pl.ds(128 * nb, nw)].astype(f32)
            if nw < 128:
                blk = jnp.concatenate([blk, jnp.zeros((D, 128 - nw), f32)], axis=1)
            tmp_v[nb, pl.ds(0, D), :] = blk
            for eb in range(5):
                rows = [tmp_v[nb, pl.ds(d, H, stride=DH), :] for d in range(4 * eb, min(4 * eb + 4, DH))]
                if len(rows) < 4:
                    rows.append(zpad)
                woT_v[pl.ds(64 * nb, nw // 2), pl.ds(128 * eb, 128)] = _to_words(jnp.concatenate(rows, axis=0).T[0:nw])

    def cols(j, start, size):
        base = j * FC + start
        return pl.ds(base if isinstance(base, int) else pl.multiple_of(base, 128), size)

    def prep_gu(j, m):
        ref = (wg_v, wu_v)[m]
        st = min(RP, 128)
        for q in range(QC // 128):
            wt = [ref[:, cols(j, s * QC + 128 * q, 128)].T for s in range(n)]
            x = [[w[:, KB * k:KB * (k + 1)].astype(f32) for k in range(n)] for w in wt]
            where = [divmod(128 * q + r0, RP) for r0 in range(0, 128, st)]
            for i, a in enumerate(_lhs_terms(x)):
                for z, (p, r) in enumerate(where):
                    a_v[term(i, QC, KB, ((2 * p + m) * RP + r) // 2, st // 2)] = _to_words(a[z * st:(z + 1) * st])
            for s in range(n):
                for z, (p, r) in enumerate(where):
                    ar_v[pl.ds(((2 * (p * n + s) + m) * RP + r) // 2, st // 2), :] = pltpu.bitcast(
                        wt[s][z * st:(z + 1) * st, 512:576], u32)

    def prep_dn(j):
        x = [[wd_v[pl.ds(RD * a, RD), cols(j, b * KD, KD)].astype(f32) for b in range(nd)] for a in range(nd)]
        for i, a in enumerate(_lhs_terms(x)):
            ad_v[term(i, RD // 2, KD, 0, RD // 2)] = _to_words(a)

    def gate_up(t, p):
        sl = pl.ds(t * W, W)
        m = [_dot(_from_words(a_v[term(i, QC, KB, p * RP, RP)]), _from_words(hb_v[pl.ds(i * KB // 2, KB // 2), sl]))
             for i in range(nm)]
        ar = _from_words(ar_v[pl.ds(p * n * RP, n * RP), :])
        r = [_dot(ar, _from_words(hr_v[pl.ds(32 * s, 32), sl])) for s in range(n)]
        c = _assemble(m)
        c = [[c[a][b] + r[b][2 * a * RP:2 * (a + 1) * RP] for b in range(n)] for a in range(n)]
        hh = [[x[0:RP] * x[RP:2 * RP] for x in row] for row in c]
        k = n // nd
        for a in range(k):
            for b in range(k):
                sub = [[hh[x * k + a][y * k + b] for y in range(nd)] for x in range(nd)]
                for i, z in enumerate(_rhs_terms(sub)):
                    g_v[term((t % 2) * nmd + i, KD // 2, WD, (a * QC + p * RP) // 2, RP // 2, b * W, W)] = _to_words(z)

    def down_term(t, i, lo, size):
        return _dot(_from_words(ad_v[term(i, RD // 2, KD, 0, RD // 2)]),
                    _from_words(g_v[term((t % 2) * nmd + i, KD // 2, WD, 0, KD // 2, lo, size)]))

    def down(t):
        for i in range(nmd):
            acc_v[pl.ds(i * RD, RD), pl.ds(t * WD, WD)] += down_term(t, i, 0, WD)

    out_copies = []

    def down_last(t):
        for b in range(WD // W):
            y = [acc_v[pl.ds(i * RD, RD), pl.ds(t * WD + b * W, W)] + down_term(t, i, b * W, W) for i in range(nmd)]
            c = _assemble(y)
            for s in range(nd):
                for u in range(W // 128):
                    col = pl.ds(128 * (n * (t * W // 128 + u) + s * (n // nd) + b), 128)
                    for a in range(nd):
                        rr = pl.ds(RD * a, RD)
                        z = x1_v[rr, col] + modc_v[pl.ds(5 * D + RD * a, RD), :] * c[a][s][:, 128 * u:128 * (u + 1)]
                        out_v[rr, col] = z.astype(bf16)
                    out_copies.append(cp(out_v.at[:, col], out_hbm.at[:, col], sems.at[next(sem_i)]))
                    out_copies[-1].start()

    copies = {}
    for item in ORDER:
        op, arg = item[0], item[1:]
        if op == '|':
            pl.semaphore_signal(bar_sem, 1)
            pl.semaphore_wait(bar_sem, 1)
        elif op == 's':
            for name in arg.split('+'):
                copies[name] = make_copies(name)
                for d in copies[name]:
                    d.start()
        elif op == 'w':
            with scope('w_' + arg):
                for name in arg.split('+'):
                    for d in copies[name]:
                        d.wait()
        elif op == 'z':
            acc_v[...] = jnp.zeros(acc_v.shape, f32)
        elif op in 'qkv':
            proj('qkv'.index(op), int(arg))
        elif op == 'a':
            attn_col(2 * int(arg))
            attn_col(2 * int(arg) + 1)
        elif op == 'b':
            attn_col(int(arg))
        elif op == 'l':
            ln1(int(arg))
        elif op == 'o':
            wo(int(arg))
        elif op == 'n':
            ln2(int(arg))
        elif op == 'g':
            gate_up(int(arg[0]), int(arg[1]))
        elif op == 'd':
            down(int(arg))
        elif op == 'p':
            if arg in 'qkv':
                prep_qkv('qkv'.index(arg))
            elif arg == 'o':
                prep_wo()
            elif arg[0] == 'd':
                prep_dn(int(arg[1]))
            else:
                prep_gu(int(arg[1]), 'gu'.index(arg[0]))
        elif op == 'm':
            mod_cols(*((0, 1152), (1152, 3456))[int(arg)])

    def chunk(j, last):
        for t in range(NFT):
            if not (last and t == NFT - 1):
                for p in range(NP):
                    gate_up((t + 1) % NFT, p)
            if t == 0:
                prep_dn(j)
            if t == NFT - 2 and not last:
                prep_gu(j + 1, 0)
                prep_gu(j + 1, 1)
            (down_last if last else down)(t)

    with scope('loop'):
        lax.fori_loop(1, NC - 1, lambda j, carry: chunk(j, False), None)
    chunk(NC - 1, True)
    with scope('w_out'):
        for d in out_copies:
            d.wait()


PRO = 'sc+q+m0+x01+k+v+x27+wo+m1+f00+f11+f28 z wq pq wc+m0 m0 wx01 l0 l1 q0 wk q1 pk wv k0 k1 pv wx27 '
PLANS = {
    0: PRO + 'v0 v1 l2 l3 q2 k2 v2 a0 a1 q3 k3 v3 a2 wwo+m1+f00+f11 '
       'm1 po l4 q4 k4 v4 o0 o1 a3 n0 pg0 pu0 l5 q5 k5 v5 G0 a4 o2 o3 n1 l6 q6 k6 v6 pd0 D0 a5 l7 q7 k7 v7 G1 a6 o4 o5 D1 a7 n2 G2 o6 o7 n3 D2 G3 pg1 pu1 D3X G0 D3 wf28',
    1: PRO + 'v0 v1 l2 l3 q2 k2 v2 a0 a1 q3 k3 v3 a2 wwo+m1+f00+f11 '
       'm1 po l4 q4 k4 v4 o0 o1 a3 n0 pg0 pu0 l5 q5 k5 v5 G0 a4 o2 o3 n1 l6 q6 k6 v6 G1 a5 pd0 l7 q7 k7 v7 D0 a6 o4 o5 n2 G2 a7 D1 o6 o7 n3 G3 pg1 pu1 D2 G0 D3 wf28',
    2: PRO + 'v0 v1 l2 l3 q2 k2 v2 a0 a1 q3 k3 wwo+m1+f00+f11 '
       'v3 a2 m1 po l4 q4 k4 v4 o0 o1 a3 n0 l5 q5 k5 v5 o2 o3 pg0 pu0 G0 a4 n1 l6 q6 k6 v6 G1 a5 pd0 l7 q7 k7 v7 D0 a6 o4 o5 n2 G2 a7 D1 o6 o7 n3 G3 pg1 pu1 D2 G0 D3 wf28',
}


def make(L=1, LD=1, NP=1, scopes=False, plan=0, ev=True):
    ORDER = []
    for item in PLANS[plan].split():
        if item[0] == 'G':
            ORDER += ['g%s%d' % (item[1], p) for p in range(NP)]
        elif item[0] == 'D':
            ORDER += [] if item[-1] == 'X' else ['d' + item[1]]
        else:
            ORDER.append(item)
    flags = {'XLA_TPU_EVENLY_DISTRIBUTE_CRITICAL_NODES': True} if ev else {}
    n, nm, nd, nmd = 2 ** L, 7 ** L, 2 ** LD, 7 ** LD

    def terms(count, per, width):
        return ((count + 1) // 2 * per, 256) if width == 128 else (count * per, width)

    @jax.jit
    def f(A_x, A_wqkv, A_wo, B_x, B_w_gate, B_w_up, B_w_down, c, w_mod):
        xT = A_x[0].T
        wdT = B_w_down.T
        hbm = pl.BlockSpec(memory_space=pltpu.HBM)
        V = pltpu.VMEM
        outT = pl.pallas_call(
            functools.partial(kernel, L=L, LD=LD, NP=NP, scopes=scopes, ORDER=ORDER),
            in_specs=[hbm] * 8,
            out_specs=hbm,
            out_shape=jax.ShapeDtypeStruct((D, S), bf16),
            scratch_shapes=[
                V((1, D), bf16), V((D, 6 * D), bf16), V((D, S), bf16), V((D, 3 * D), bf16), V((D, D), bf16),
                V((5, 3 * D, 128), f32), V((3 * D // 2, 640), u32), V((D // 2, 640), u32), V((6 * D, 128), f32),
                V((D // 2, S), u32), V((D // 2, S), u32), V((D // 2, S + 128), u32), V((D // 2, S + 128), u32),
                V((D // 2, S), u32), V((D, S), f32), V((nm * 256 // n, S // n), u32), V((n * 32, S // n), u32),
                V((D, F), bf16), V((D, F), bf16), V((D, F), bf16),
                V(terms(nm, FC // n, 512 // n), u32), V((FC, 64), u32), V(terms(nmd, D // nd // 2, FC // nd), u32),
                V(terms(2 * nmd, FC // nd // 2, 512 // nd), u32), V((nmd * D // nd, S // nd), f32), V((D, S), bf16),
                pltpu.SemaphoreType.DMA((48,)), pltpu.SemaphoreType.REGULAR,
            ],
            compiler_params=pltpu.CompilerParams(flags=flags, vmem_limit_bytes=120 * 1024 * 1024),
        )(xT, A_wqkv, A_wo, B_w_gate, B_w_up, wdT, c, w_mod)
        return outT.T[None]
    return f


pallas_adaLN_cond__sliding_local_dilated__glu_gated_bilinear__prompt_kernel = make(L=2, LD=2, NP=4, plan=1)
```

```python
import contextlib
import functools
import jax
import jax.numpy as jnp
from jax import lax
import jax.experimental.pallas as pl
import jax.experimental.pallas.tpu as pltpu

D, H, DH, WIN, DIL, F, S = 576, 32, 18, 8, 2, 4608, 2048
EPS = 1e-5
f32, bf16, u32 = jnp.float32, jnp.bfloat16, jnp.uint32
TN = 256
NT = S // TN
FC = 512
NC = F // FC


def _dot(a, b):
    return jnp.dot(a, b, preferred_element_type=f32)


def _to_words(x):
    return pltpu.bitcast(x.astype(bf16), u32)


def _from_words(x):
    return pltpu.bitcast(x, bf16)


def _halves(x):
    return tuple(pltpu.unpack_elementwise(x, index=i, packed_dtype=bf16, unpacked_dtype=f32) for i in range(2))


def _add(x, y):
    return [[a + b for a, b in zip(r, s)] for r, s in zip(x, y)]


def _sub(x, y):
    return [[a - b for a, b in zip(r, s)] for r, s in zip(x, y)]


def _quad(x):
    h = len(x) // 2
    return [r[:h] for r in x[:h]], [r[h:] for r in x[:h]], [r[:h] for r in x[h:]], [r[h:] for r in x[h:]]


def _lhs_terms(x):
    if len(x) == 1:
        return [x[0][0]]
    a11, a12, a21, a22 = _quad(x)
    terms = (_add(a11, a22), _add(a21, a22), a11, a22, _add(a11, a12), _sub(a21, a11), _sub(a12, a22))
    return [z for y in terms for z in _lhs_terms(y)]


def _rhs_terms(x):
    if len(x) == 1:
        return [x[0][0]]
    b11, b12, b21, b22 = _quad(x)
    terms = (_add(b11, b22), b11, _sub(b12, b22), _sub(b21, b11), b22, _add(b11, b12), _add(b21, b22))
    return [z for y in terms for z in _rhs_terms(y)]


def _assemble(m):
    if len(m) == 1:
        return [[m[0]]]
    n = len(m) // 7
    p = [_assemble(m[i * n:(i + 1) * n]) for i in range(7)]
    c11 = _add(_sub(_add(p[0], p[3]), p[4]), p[6])
    c12 = _add(p[2], p[4])
    c21 = _add(p[1], p[3])
    c22 = _add(_add(_sub(p[0], p[1]), p[2]), p[5])
    return [a + b for a, b in zip(c11, c12)] + [a + b for a, b in zip(c21, c22)]


def _col_mean(x):
    r = x.shape[0] // 4
    return jnp.sum((x[0:r] + x[r:2 * r]) + (x[2 * r:3 * r] + x[3 * r:]), axis=0, keepdims=True) * (1.0 / D)


def _ln_mod(x, scale, shift):
    xc = x - _col_mean(x)
    return xc * lax.rsqrt(_col_mean(xc * xc) + EPS) * scale + shift


def kernel(xT_hbm, wqkv_hbm, wo_hbm, wg_hbm, wu_hbm, wdT_hbm, c_hbm, wmod_hbm, out_hbm,
           c_v, wmod_v, x_v, wqkv_v, wo_v, tmp_v, wqkvT_v, woT_v, modc_v,
           h_v, q_v, k_v, v_v, o_v, x1_v, stat_v, hb_v, hr_v, wg_v, wu_v, wd_v, a_v, ar_v, ad_v, g_v, acc_v, out_v,
           sems, bar_sem, *, L, LD, NP, scopes, ORDER, SHORT):
    n, nm, nd, nmd = 2 ** L, 7 ** L, 2 ** LD, 7 ** LD
    QC, KB, RD, KD = FC // n, 512 // n, D // nd, FC // nd
    W = 512 // n
    NFT = S // (n * W)
    WD = W * n // nd
    RP = QC // NP
    cp = pltpu.make_async_copy
    scope = jax.named_scope if scopes else (lambda name: contextlib.nullcontext())
    sem_i = iter(range(64))

    def colcp(src, dst, lo, hi):
        return cp(src.at[:, pl.ds(lo, hi - lo)], dst.at[:, pl.ds(lo, hi - lo)], sems.at[next(sem_i)])

    def make_copies(name):
        if name[0] == 'x':
            return [colcp(xT_hbm, x_v, int(name[1]) * TN, (int(name[2]) + 1) * TN)]
        if name[0] == 'f':
            return [colcp(s, d, int(name[1]) * FC, (int(name[2]) + 1) * FC)
                    for s, d in ((wg_hbm, wg_v), (wu_hbm, wu_v), (wdT_hbm, wd_v))]
        if name == 'c':
            return [cp(c_hbm, c_v, sems.at[next(sem_i)])]
        if name == 'wo':
            return [cp(wo_hbm, wo_v, sems.at[next(sem_i)])]
        if name[0] == 'm':
            return [colcp(wmod_hbm, wmod_v, *((0, 1152), (1152, 3456))[int(name[1])])]
        return [colcp(wqkv_hbm, wqkv_v, *{'q': (0, 640), 'k': (640, 1152), 'v': (1152, 1728)}[name])]

    def mod_cols(lo, hi):
        cc = c_v[...].astype(f32)
        sc = jnp.broadcast_to(cc * jax.nn.sigmoid(cc), (16, D)).astype(bf16)
        m = _dot(sc, wmod_v[:, pl.ds(lo, hi - lo)])[0:8]
        lane = lo + lax.broadcasted_iota(jnp.int32, m.shape, 1)
        one = ((lane >= D) & (lane < 2 * D)) | ((lane >= 4 * D) & (lane < 5 * D))
        m = m + jnp.where(one, 1.0, 0.0)
        for j in range((hi - lo) // 128):
            blk = jnp.tile(m[:, 128 * j:128 * (j + 1)], (16, 1))
            modc_v[pl.ds(lo + 128 * j, 128), :] = blk.T

    def mod(i):
        return modc_v[pl.ds(i * D, D), :]

    def ln1(t):
        for j in range(2 * t, 2 * t + 2):
            c = pl.ds(128 * j, 128)
            h_v[:, c] = _to_words(_ln_mod(x_v[:, c].astype(f32), mod(1), mod(0)))

    def ln1_stats(t):
        for j in range(2 * t, 2 * t + 2):
            c = pl.ds(128 * j, 128)
            x = x_v[:, c].astype(f32)
            m = _col_mean(x)
            xc = x - m
            stat_v[16:24, c] = jnp.broadcast_to(m, (8, 128))
            stat_v[24:32, c] = jnp.broadcast_to(lax.rsqrt(_col_mean(xc * xc) + EPS), (8, 128))

    def ln1_apply(t):
        for j in range(2 * t, 2 * t + 2):
            c = pl.ds(128 * j, 128)
            h_v[:, c] = _to_words((x_v[:, c].astype(f32) - stat_v[16:17, c]) * stat_v[24:25, c] * mod(1) + mod(0))

    zpad = jnp.zeros((64, 128), f32)

    def prep_qkv(p):
        for kb in range(5):
            kw = min(128, D - 128 * kb)
            for j in ((0, 1, 2, 3, 4), (5, 6, 7, 8), (9, 10, 11, 12, 13))[p]:
                w = min(128, 3 * D - 128 * j)
                blk = wqkv_v[pl.ds(128 * kb, kw), pl.ds(128 * j, w)].astype(f32)
                if w < 128:
                    blk = jnp.concatenate([blk, jnp.zeros((kw, 128 - w), f32)], axis=1)
                if kw < 128:
                    blk = jnp.concatenate([blk, zpad], axis=0)
                tmp_v[kb, pl.ds(128 * j, w), :] = blk.T[0:w]
            for d in range(DH):
                r = tmp_v[kb, pl.ds(p * D + d, H, stride=DH), :]
                wqkvT_v[pl.ds((p * D + d * H) // 2, H // 2), pl.ds(128 * kb, 128)] = _to_words(r)

    def proj(p, t):
        w = _from_words(wqkvT_v[pl.ds(p * D // 2, D // 2), :])[:, 0:D]
        y = _to_words(_dot(w, _from_words(h_v[:, pl.ds(t * TN, TN)])))
        if p == 0:
            q_v[:, pl.ds(t * TN, TN)] = y
        else:
            ref = (k_v, v_v)[p - 1]
            ref[:, pl.ds(128 + t * TN, TN)] = y
            if t == 0:
                ref[:, pl.ds(0, 128)] = jnp.broadcast_to(y[:, 0:1], (D // 2, 128))

    lane = lax.broadcasted_iota(jnp.int32, (8, 128), 1)
    scale = DH ** -0.5

    def window(ref, r, j):
        cur = ref[pl.ds(r, 8), pl.ds(128 * (j + 1), 128)]
        prev = ref[pl.ds(r, 8), pl.ds(128 * j, 128)]
        yield _halves(cur)
        for w in range(1, WIN):
            yield _halves(pltpu.roll(jnp.where(lane < 128 - DIL * w, cur, prev), DIL * w, 1))

    def attn_col(j):
        c = pl.ds(128 * j, 128)
        for hg in range(2):
            lg = [[None] * WIN, [None] * WIN]
            for d in range(DH):
                r = d * (H // 2) + hg * 8
                q = _halves(q_v[pl.ds(r, 8), c])
                for w, k in enumerate(window(k_v, r, j)):
                    for s in range(2):
                        pr = q[s] * k[s]
                        lg[s][w] = pr if d == 0 else lg[s][w] + pr
            p = []
            for s in range(2):
                l = [x * scale for x in lg[s]]
                if j == 0:
                    l = [x if w == 0 else jnp.where(lane >= DIL * w, x, -1e9) for w, x in enumerate(l)]
                mx = functools.reduce(jnp.maximum, l)
                e = [jnp.exp(x - mx) for x in l]
                inv = 1.0 / functools.reduce(lambda a, b: a + b, e)
                p.append([x * inv for x in e])
            for d in range(DH):
                r = d * (H // 2) + hg * 8
                o = [None, None]
                for w, v in enumerate(window(v_v, r, j)):
                    for s in range(2):
                        pr = p[s][w] * v[s]
                        o[s] = pr if w == 0 else o[s] + pr
                o_v[pl.ds(r, 8), c] = pltpu.pack_elementwise(o, packed_dtype=bf16)

    def wo(t):
        y = _dot(_from_words(woT_v[...])[:, 0:D], _from_words(o_v[:, pl.ds(t * TN, TN)]))
        for s in range(2):
            c = pl.ds(t * TN + 128 * s, 128)
            x1 = x_v[:, c].astype(f32) + mod(2) * y[:, 128 * s:128 * (s + 1)]
            x1_v[:, c] = x1
            dev = x1 - x1[0:1]
            m = jnp.sum(dev, axis=0, keepdims=True) * (1.0 / D)
            var = jnp.sum(dev * dev, axis=0, keepdims=True) * (1.0 / D) - m * m
            stat_v[0:8, c] = jnp.broadcast_to(m + x1[0:1], (8, 128))
            stat_v[8:16, c] = jnp.broadcast_to(var, (8, 128))

    def term(i, per, width, r0, nr, c0=0, nc=None):
        k = 2 if width == 128 else 1
        return pl.ds((i // k) * per + r0, nr), pl.ds((i % k) * width + c0, width if nc is None else nc)

    def ln2(u):
        h2 = []
        for s in range(n):
            c = pl.ds(128 * (n * u + s), 128)
            rstd = lax.rsqrt(jnp.maximum(stat_v[8:9, c], 0.0) + EPS)
            h2.append((x1_v[:, c] - stat_v[0:1, c]) * rstd * mod(4) + mod(3))
        c = pl.ds(128 * u, 128)
        for i, b in enumerate(_rhs_terms([[h2[s][KB * k:KB * (k + 1)] for s in range(n)] for k in range(n)])):
            hb_v[pl.ds(i * KB // 2, KB // 2), c] = _to_words(b)
        for s in range(n):
            hr_v[pl.ds(32 * s, 32), c] = _to_words(h2[s][512:576])

    def prep_wo():
        for nb in range(5):
            nw = min(128, D - 128 * nb)
            blk = wo_v[:, pl.ds(128 * nb, nw)].astype(f32)
            if nw < 128:
                blk = jnp.concatenate([blk, jnp.zeros((D, 128 - nw), f32)], axis=1)
            tmp_v[nb, pl.ds(0, D), :] = blk
            for eb in range(5):
                rows = [tmp_v[nb, pl.ds(d, H, stride=DH), :] for d in range(4 * eb, min(4 * eb + 4, DH))]
                if len(rows) < 4:
                    rows.append(zpad)
                woT_v[pl.ds(64 * nb, nw // 2), pl.ds(128 * eb, 128)] = _to_words(jnp.concatenate(rows, axis=0).T[0:nw])

    def cols(j, start, size):
        base = j * FC + start
        return pl.ds(base if isinstance(base, int) else pl.multiple_of(base, 128), size)

    def prep_gu(j, m):
        ref = (wg_v, wu_v)[m]
        st = min(RP, 128)
        for q in range(QC // 128):
            wt = [ref[:, cols(j, s * QC + 128 * q, 128)].T for s in range(n)]
            x = [[w[:, KB * k:KB * (k + 1)].astype(f32) for k in range(n)] for w in wt]
            where = [divmod(128 * q + r0, RP) for r0 in range(0, 128, st)]
            for i, a in enumerate(_lhs_terms(x)):
                for z, (p, r) in enumerate(where):
                    a_v[term(i, QC, KB, ((2 * p + m) * RP + r) // 2, st // 2)] = _to_words(a[z * st:(z + 1) * st])
            for s in range(n):
                for z, (p, r) in enumerate(where):
                    ar_v[pl.ds(((2 * (p * n + s) + m) * RP + r) // 2, st // 2), :] = pltpu.bitcast(
                        wt[s][z * st:(z + 1) * st, 512:576], u32)

    def prep_dn(j):
        x = [[wd_v[pl.ds(RD * a, RD), cols(j, b * KD, KD)].astype(f32) for b in range(nd)] for a in range(nd)]
        for i, a in enumerate(_lhs_terms(x)):
            ad_v[term(i, RD // 2, KD, 0, RD // 2)] = _to_words(a)

    def gate_up(t, p):
        sl = pl.ds(t * W, W)
        m = [_dot(_from_words(a_v[term(i, QC, KB, p * RP, RP)]), _from_words(hb_v[pl.ds(i * KB // 2, KB // 2), sl]))
             for i in range(nm)]
        ar = _from_words(ar_v[pl.ds(p * n * RP, n * RP), :])
        r = [_dot(ar, _from_words(hr_v[pl.ds(32 * s, 32), sl])) for s in range(n)]
        c = _assemble(m)
        c = [[c[a][b] + r[b][2 * a * RP:2 * (a + 1) * RP] for b in range(n)] for a in range(n)]
        hh = [[x[0:RP] * x[RP:2 * RP] for x in row] for row in c]
        k = n // nd
        for a in range(k):
            for b in range(k):
                sub = [[hh[x * k + a][y * k + b] for y in range(nd)] for x in range(nd)]
                for i, z in enumerate(_rhs_terms(sub)):
                    g_v[term((t % 2) * nmd + i, KD // 2, WD, (a * QC + p * RP) // 2, RP // 2, b * W, W)] = _to_words(z)

    def down_term(t, i, lo, size):
        return _dot(_from_words(ad_v[term(i, RD // 2, KD, 0, RD // 2)]),
                    _from_words(g_v[term((t % 2) * nmd + i, KD // 2, WD, 0, KD // 2, lo, size)]))

    def down(t):
        for i in range(nmd):
            acc_v[pl.ds(i * RD, RD), pl.ds(t * WD, WD)] += down_term(t, i, 0, WD)

    out_copies = []

    def down_last(t):
        per, half = nmd // 7, nd // 2
        for b in range(WD // W):
            part = {}

            def emit(qa, qb, c):
                for s in range(half):
                    for u in range(W // 128):
                        col = pl.ds(128 * (n * (t * W // 128 + u) + (qb * half + s) * (n // nd) + b), 128)
                        for a in range(half):
                            r0 = RD * (qa * half + a)
                            z = c[a][s][:, 128 * u:128 * (u + 1)]
                            out_v[pl.ds(r0, RD), col] = (
                                x1_v[pl.ds(r0, RD), col] + modc_v[pl.ds(5 * D + r0, RD), :] * z).astype(bf16)
                        rr = pl.ds(qa * D // 2, D // 2)
                        out_copies.append(cp(out_v.at[rr, col], out_hbm.at[rr, col], sems.at[next(sem_i)]))
                        out_copies[-1].start()

            for g in (1, 3, 2, 4, 0, 6, 5):
                part[g] = _assemble([acc_v[pl.ds(i * RD, RD), pl.ds(t * WD + b * W, W)] + down_term(t, i, b * W, W)
                                     for i in range(g * per, (g + 1) * per)])
                if g == 3:
                    emit(1, 0, _add(part[1], part[3]))
                elif g == 4:
                    emit(0, 1, _add(part[2], part[4]))
                elif g == 6:
                    emit(0, 0, _add(_sub(_add(part[0], part[3]), part[4]), part[6]))
                elif g == 5:
                    emit(1, 1, _add(_add(_sub(part[0], part[1]), part[2]), part[5]))

    copies = {}
    for item in ORDER:
        op, arg = item[0], item[1:]
        if op == '|':
            pl.semaphore_signal(bar_sem, 1)
            pl.semaphore_wait(bar_sem, 1)
        elif op == 's':
            for name in arg.split('+'):
                copies[name] = make_copies(name)
                for d in copies[name]:
                    d.start()
        elif op == 'w':
            with scope('w_' + arg):
                for name in arg.split('+'):
                    for d in copies[name]:
                        d.wait()
        elif op == 'z':
            acc_v[...] = jnp.zeros(acc_v.shape, f32)
        elif op in 'qkv':
            proj('qkv'.index(op), int(arg))
        elif op == 'a':
            attn_col(2 * int(arg))
            attn_col(2 * int(arg) + 1)
        elif op == 'b':
            attn_col(int(arg))
        elif op == 'l':
            ln1(int(arg))
        elif op == 'S':
            ln1_stats(int(arg))
        elif op == 'N':
            ln1_apply(int(arg))
        elif op == 'o':
            wo(int(arg))
        elif op == 'n':
            ln2(int(arg))
        elif op == 'g':
            gate_up(int(arg[0]), int(arg[1]))
        elif op == 'd':
            down(int(arg))
        elif op == 'p':
            if arg in 'qkv':
                prep_qkv('qkv'.index(arg))
            elif arg == 'o':
                prep_wo()
            elif arg[0] == 'd':
                prep_dn(int(arg[1]))
            else:
                prep_gu(int(arg[1]), 'gu'.index(arg[0]))
        elif op == 'm':
            mod_cols(*((0, 1152), (1152, 3456))[int(arg)])

    def chunk(j, last):
        for t in range(NFT):
            if not (last and t == NFT - 1):
                for p in range(NP):
                    gate_up((t + 1) % NFT, p)
            if t == 0:
                prep_dn(j)
            if t == NFT - 2 and not last:
                prep_gu(j + 1, 0)
                prep_gu(j + 1, 1)
            (down_last if last else down)(t)

    if SHORT:
        def keep(j, carry):
            r = pl.ds(pl.multiple_of(j * 8, 8), 8)
            z = acc_v[r, 0:128]
            for ref in (a_v, ad_v, g_v, hb_v, hr_v):
                z = z + pltpu.bitcast(ref[r, 0:128], f32)
            z = z + x1_v[r, 0:128] + modc_v[r, :]
            z = z + jnp.tile(pltpu.bitcast(ar_v[r, :], f32), (1, 2))
            x1_v[r, 0:128] = z
            return carry
        lax.fori_loop(0, 4, keep, None)
        out_v[0:16, 0:128] = x1_v[0:16, 0:128].astype(bf16)
        d = cp(out_v, out_hbm, sems.at[next(sem_i)])
        d.start()
        d.wait()
        return
    with scope('loop'):
        lax.fori_loop(1, NC - 1, lambda j, carry: chunk(j, False), None)
    chunk(NC - 1, True)
    with scope('w_out'):
        for d in out_copies:
            d.wait()


PRO = 'sc+q+x01+m0+k+v+x27+wo+m1+f00+f11+f28 z wq pq wx01 S0 S1 wc+m0 m0 N0 N1 q0 wk q1 pk wv k0 k1 pv wx27+wo '
PLANS = {
    0: PRO + 'v0,v1,l2,l3,q2,k2,v2,a0,a1,q3,k3,v3,l4,a2,po,wm1+f00+f11,m1,o0,o1,l5,q4,k4,v4,a3,n0,pg0,pu0,o2,o3,l6,q5,k5,v5,'
             'G0,a4,n1,l7,q6,k6,v6,G1,a5,pd0,o4,q7,k7,v7,a6,o5,n2,D0,G2,a7,o6,o7,D1,n3,g30,|,g31,g32,g33,pg1,pu1,D2,G0,D3,wf28'.replace(',', ' '),
}


def make(L=1, LD=1, NP=1, scopes=False, plan=0, ev=True, short=False):
    ORDER = []
    for item in (PLANS[plan] if isinstance(plan, int) else PRO + plan.replace(',', ' ')).split():
        if item[0] == 'G':
            ORDER += ['g%s%d' % (item[1], p) for p in range(NP)]
        elif item[0] == 'D':
            ORDER += [] if item[-1] == 'X' else ['d' + item[1]]
        else:
            ORDER.append(item)
    flags = {'XLA_TPU_EVENLY_DISTRIBUTE_CRITICAL_NODES': True} if ev else {}
    n, nm, nd, nmd = 2 ** L, 7 ** L, 2 ** LD, 7 ** LD

    def terms(count, per, width):
        return ((count + 1) // 2 * per, 256) if width == 128 else (count * per, width)

    @jax.jit
    def f(A_x, A_wqkv, A_wo, B_x, B_w_gate, B_w_up, B_w_down, c, w_mod):
        xT = A_x[0].T
        wdT = B_w_down.T
        hbm = pl.BlockSpec(memory_space=pltpu.HBM)
        V = pltpu.VMEM
        outT = pl.pallas_call(
            functools.partial(kernel, L=L, LD=LD, NP=NP, scopes=scopes, ORDER=ORDER, SHORT=short),
            in_specs=[hbm] * 8,
            out_specs=hbm,
            out_shape=jax.ShapeDtypeStruct((D, S), bf16),
            scratch_shapes=[
                V((1, D), bf16), V((D, 6 * D), bf16), V((D, S), bf16), V((D, 3 * D), bf16), V((D, D), bf16),
                V((5, 3 * D, 128), f32), V((3 * D // 2, 640), u32), V((D // 2, 640), u32), V((6 * D, 128), f32),
                V((D // 2, S), u32), V((D // 2, S), u32), V((D // 2, S + 128), u32), V((D // 2, S + 128), u32),
                V((D // 2, S), u32), V((D, S), f32), V((32, S), f32), V((nm * 256 // n, S // n), u32), V((n * 32, S // n), u32),
                V((D, F), bf16), V((D, F), bf16), V((D, F), bf16),
                V(terms(nm, FC // n, 512 // n), u32), V((FC, 64), u32), V(terms(nmd, D // nd // 2, FC // nd), u32),
                V(terms(2 * nmd, FC // nd // 2, 512 // nd), u32), V((nmd * D // nd, S // nd), f32), V((D, S), bf16),
                pltpu.SemaphoreType.DMA((64,)), pltpu.SemaphoreType.REGULAR,
            ],
            compiler_params=pltpu.CompilerParams(flags=flags, vmem_limit_bytes=120 * 1024 * 1024),
        )(xT, A_wqkv, A_wo, B_w_gate, B_w_up, wdT, c, w_mod)
        return outT.T[None]
    return f


pallas_adaLN_cond__sliding_local_dilated__glu_gated_bilinear__prompt_kernel = make(L=2, LD=2, NP=4)
```

```python
import contextlib
import functools
import jax
import jax.numpy as jnp
from jax import lax
import jax.experimental.pallas as pl
import jax.experimental.pallas.tpu as pltpu

D, H, DH, WIN, DIL, F, S = 576, 32, 18, 8, 2, 4608, 2048
EPS = 1e-5
f32, bf16, u32 = jnp.float32, jnp.bfloat16, jnp.uint32
TN = 256
NT = S // TN
FC = 512
NC = F // FC


def _dot(a, b):
    return jnp.dot(a, b, preferred_element_type=f32)


def _to_words(x):
    return pltpu.bitcast(x.astype(bf16), u32)


def _from_words(x):
    return pltpu.bitcast(x, bf16)


def _halves(x):
    return tuple(pltpu.unpack_elementwise(x, index=i, packed_dtype=bf16, unpacked_dtype=f32) for i in range(2))


def _add(x, y):
    return [[a + b for a, b in zip(r, s)] for r, s in zip(x, y)]


def _sub(x, y):
    return [[a - b for a, b in zip(r, s)] for r, s in zip(x, y)]


def _quad(x):
    h = len(x) // 2
    return [r[:h] for r in x[:h]], [r[h:] for r in x[:h]], [r[:h] for r in x[h:]], [r[h:] for r in x[h:]]


def _lhs_terms(x):
    if len(x) == 1:
        return [x[0][0]]
    a11, a12, a21, a22 = _quad(x)
    terms = (_add(a11, a22), _add(a21, a22), a11, a22, _add(a11, a12), _sub(a21, a11), _sub(a12, a22))
    return [z for y in terms for z in _lhs_terms(y)]


def _rhs_terms(x):
    if len(x) == 1:
        return [x[0][0]]
    b11, b12, b21, b22 = _quad(x)
    terms = (_add(b11, b22), b11, _sub(b12, b22), _sub(b21, b11), b22, _add(b11, b12), _add(b21, b22))
    return [z for y in terms for z in _rhs_terms(y)]


def _assemble(m):
    if len(m) == 1:
        return [[m[0]]]
    n = len(m) // 7
    p = [_assemble(m[i * n:(i + 1) * n]) for i in range(7)]
    c11 = _add(_sub(_add(p[0], p[3]), p[4]), p[6])
    c12 = _add(p[2], p[4])
    c21 = _add(p[1], p[3])
    c22 = _add(_add(_sub(p[0], p[1]), p[2]), p[5])
    return [a + b for a, b in zip(c11, c12)] + [a + b for a, b in zip(c21, c22)]


def _col_mean(x):
    r = x.shape[0] // 4
    return jnp.sum((x[0:r] + x[r:2 * r]) + (x[2 * r:3 * r] + x[3 * r:]), axis=0, keepdims=True) * (1.0 / D)


def _ln_mod(x, scale, shift):
    xc = x - _col_mean(x)
    return xc * lax.rsqrt(_col_mean(xc * xc) + EPS) * scale + shift


def kernel(xT_hbm, wqkv_hbm, wo_hbm, wg_hbm, wu_hbm, wdT_hbm, c_hbm, wmod_hbm, out_hbm,
           c_v, wmod_v, x_v, wqkv_v, wo_v, tmp_v, wqkvT_v, woT_v, modc_v,
           h_v, q_v, k_v, v_v, o_v, x1_v, stat_v, hb_v, hr_v, wg_v, wu_v, wd_v, wt_v, a_v, ar_v, ad_v, g_v, acc_v, out_v,
           sems, bar_sem, *, L, LD, NP, scopes, ORDER, SHORT, SL, UN, BULK):
    n, nm, nd, nmd = 2 ** L, 7 ** L, 2 ** LD, 7 ** LD
    QC, KB, RD, KD = FC // n, 512 // n, D // nd, FC // nd
    W = 512 // n
    NFT = S // (n * W)
    WD = W * n // nd
    RP = QC // NP
    cp = pltpu.make_async_copy
    scope = jax.named_scope if scopes else (lambda name: contextlib.nullcontext())
    sem_i = iter(range(64))

    def colcp(src, dst, lo, hi):
        return cp(src.at[:, pl.ds(lo, hi - lo)], dst.at[:, pl.ds(lo, hi - lo)], sems.at[next(sem_i)])

    def make_copies(name):
        if name[0] == 'x':
            return [colcp(xT_hbm, x_v, int(name[1]) * TN, (int(name[2]) + 1) * TN)]
        if name[0] == 'f':
            return [colcp(s, d, int(name[1]) * FC, (int(name[2]) + 1) * FC)
                    for s, d in ((wg_hbm, wg_v), (wu_hbm, wu_v), (wdT_hbm, wd_v))]
        if name == 'c':
            return [cp(c_hbm, c_v, sems.at[next(sem_i)])]
        if name == 'wo':
            return [cp(wo_hbm, wo_v, sems.at[next(sem_i)])]
        if name[0] == 'm':
            return [colcp(wmod_hbm, wmod_v, *((0, 1152), (1152, 3456))[int(name[1])])]
        return [colcp(wqkv_hbm, wqkv_v, *{'q': (0, 640), 'k': (640, 1152), 'v': (1152, 1728)}[name])]

    def mod_cols(lo, hi):
        cc = c_v[...].astype(f32)
        sc = jnp.broadcast_to(cc * jax.nn.sigmoid(cc), (16, D)).astype(bf16)
        m = _dot(sc, wmod_v[:, pl.ds(lo, hi - lo)])[0:8]
        lane = lo + lax.broadcasted_iota(jnp.int32, m.shape, 1)
        one = ((lane >= D) & (lane < 2 * D)) | ((lane >= 4 * D) & (lane < 5 * D))
        m = m + jnp.where(one, 1.0, 0.0)
        for j in range((hi - lo) // 128):
            blk = jnp.tile(m[:, 128 * j:128 * (j + 1)], (16, 1))
            modc_v[pl.ds(lo + 128 * j, 128), :] = blk.T

    def mod(i):
        return modc_v[pl.ds(i * D, D), :]

    def ln1(t):
        for j in range(2 * t, 2 * t + 2):
            c = pl.ds(128 * j, 128)
            h_v[:, c] = _to_words(_ln_mod(x_v[:, c].astype(f32), mod(1), mod(0)))

    def ln1_stats(t):
        for j in range(2 * t, 2 * t + 2):
            c = pl.ds(128 * j, 128)
            x = x_v[:, c].astype(f32)
            m = _col_mean(x)
            xc = x - m
            stat_v[16:24, c] = jnp.broadcast_to(m, (8, 128))
            stat_v[24:32, c] = jnp.broadcast_to(lax.rsqrt(_col_mean(xc * xc) + EPS), (8, 128))

    def ln1_apply(t):
        for j in range(2 * t, 2 * t + 2):
            c = pl.ds(128 * j, 128)
            h_v[:, c] = _to_words((x_v[:, c].astype(f32) - stat_v[16:17, c]) * stat_v[24:25, c] * mod(1) + mod(0))

    zpad = jnp.zeros((64, 128), f32)

    def prep_qkv(p):
        for kb in range(5):
            kw = min(128, D - 128 * kb)
            for j in ((0, 1, 2, 3, 4), (5, 6, 7, 8), (9, 10, 11, 12, 13))[p]:
                w = min(128, 3 * D - 128 * j)
                blk = wqkv_v[pl.ds(128 * kb, kw), pl.ds(128 * j, w)].astype(f32)
                if w < 128:
                    blk = jnp.concatenate([blk, jnp.zeros((kw, 128 - w), f32)], axis=1)
                if kw < 128:
                    blk = jnp.concatenate([blk, zpad], axis=0)
                tmp_v[kb, pl.ds(128 * j, w), :] = blk.T[0:w]
            for d in range(DH):
                r = tmp_v[kb, pl.ds(p * D + d, H, stride=DH), :]
                wqkvT_v[pl.ds((p * D + d * H) // 2, H // 2), pl.ds(128 * kb, 128)] = _to_words(r)

    def proj(p, t):
        w = _from_words(wqkvT_v[pl.ds(p * D // 2, D // 2), :])[:, 0:D]
        y = _to_words(_dot(w, _from_words(h_v[:, pl.ds(t * TN, TN)])))
        if p == 0:
            q_v[:, pl.ds(t * TN, TN)] = y
        else:
            ref = (k_v, v_v)[p - 1]
            ref[:, pl.ds(128 + t * TN, TN)] = y
            if t == 0:
                ref[:, pl.ds(0, 128)] = jnp.broadcast_to(y[:, 0:1], (D // 2, 128))

    lane = lax.broadcasted_iota(jnp.int32, (8, 128), 1)
    scale = DH ** -0.5

    def window(ref, r, j):
        cur = ref[pl.ds(r, 8), pl.ds(128 * (j + 1), 128)]
        prev = ref[pl.ds(r, 8), pl.ds(128 * j, 128)]
        yield _halves(cur)
        for w in range(1, WIN):
            yield _halves(pltpu.roll(jnp.where(lane < 128 - DIL * w, cur, prev), DIL * w, 1))

    def attn_col(j):
        c = pl.ds(128 * j, 128)
        for hg in range(2):
            lg = [[None] * WIN, [None] * WIN]
            for d in range(DH):
                r = d * (H // 2) + hg * 8
                q = _halves(q_v[pl.ds(r, 8), c])
                for w, k in enumerate(window(k_v, r, j)):
                    for s in range(2):
                        pr = q[s] * k[s]
                        lg[s][w] = pr if d == 0 else lg[s][w] + pr
            p = []
            for s in range(2):
                l = [x * scale for x in lg[s]]
                if j == 0:
                    l = [x if w == 0 else jnp.where(lane >= DIL * w, x, -1e9) for w, x in enumerate(l)]
                mx = functools.reduce(jnp.maximum, l)
                e = [jnp.exp(x - mx) for x in l]
                inv = 1.0 / functools.reduce(lambda a, b: a + b, e)
                p.append([x * inv for x in e])
            for d in range(DH):
                r = d * (H // 2) + hg * 8
                o = [None, None]
                for w, v in enumerate(window(v_v, r, j)):
                    for s in range(2):
                        pr = p[s][w] * v[s]
                        o[s] = pr if w == 0 else o[s] + pr
                o_v[pl.ds(r, 8), c] = pltpu.pack_elementwise(o, packed_dtype=bf16)

    def wo(t):
        y = _dot(_from_words(woT_v[...])[:, 0:D], _from_words(o_v[:, pl.ds(t * TN, TN)]))
        for s in range(2):
            c = pl.ds(t * TN + 128 * s, 128)
            x1 = x_v[:, c].astype(f32) + mod(2) * y[:, 128 * s:128 * (s + 1)]
            x1_v[:, c] = x1
            dev = x1 - x1[0:1]
            m = jnp.sum(dev, axis=0, keepdims=True) * (1.0 / D)
            var = jnp.sum(dev * dev, axis=0, keepdims=True) * (1.0 / D) - m * m
            stat_v[0:8, c] = jnp.broadcast_to(m + x1[0:1], (8, 128))
            stat_v[8:16, c] = jnp.broadcast_to(var, (8, 128))

    def term(i, per, width, r0, nr, c0=0, nc=None):
        k = 2 if width == 128 else 1
        return pl.ds((i // k) * per + r0, nr), pl.ds((i % k) * width + c0, width if nc is None else nc)

    def ln2(u):
        cs = [pl.ds(128 * (n * u + s), 128) for s in range(n)]
        mean = [stat_v[0:1, c] for c in cs]
        rstd = [lax.rsqrt(jnp.maximum(stat_v[8:9, c], 0.0) + EPS) for c in cs]

        def h2(r0, nr, s):
            return ((x1_v[pl.ds(r0, nr), cs[s]] - mean[s]) * rstd[s] * modc_v[pl.ds(4 * D + r0, nr), :]
                    + modc_v[pl.ds(3 * D + r0, nr), :])

        c = pl.ds(128 * u, 128)
        for r0 in range(0, KB, SL):
            for i, b in enumerate(_rhs_terms([[h2(KB * k + r0, SL, s) for s in range(n)] for k in range(n)])):
                hb_v[pl.ds((i * KB + r0) // 2, SL // 2), c] = _to_words(b)
        for s in range(n):
            hr_v[pl.ds(32 * s, 32), c] = _to_words(h2(512, 64, s))

    def prep_wo():
        for nb in range(5):
            nw = min(128, D - 128 * nb)
            blk = wo_v[:, pl.ds(128 * nb, nw)].astype(f32)
            if nw < 128:
                blk = jnp.concatenate([blk, jnp.zeros((D, 128 - nw), f32)], axis=1)
            tmp_v[nb, pl.ds(0, D), :] = blk
            for eb in range(5):
                rows = [tmp_v[nb, pl.ds(d, H, stride=DH), :] for d in range(4 * eb, min(4 * eb + 4, DH))]
                if len(rows) < 4:
                    rows.append(zpad)
                woT_v[pl.ds(64 * nb, nw // 2), pl.ds(128 * eb, 128)] = _to_words(jnp.concatenate(rows, axis=0).T[0:nw])

    def cols(j, start, size):
        base = j * FC + start
        return pl.ds(base if isinstance(base, int) else pl.multiple_of(base, 128), size)

    def weight_rows(j, m, q):
        return (wg_v, wu_v)[m][:, cols(j, 128 * q, 128)].T

    def transpose_gu(j):
        for m in range(2):
            for q in range(FC // 128):
                wt_v[pl.ds((m * FC + 128 * q) // 2, 64), 0:D] = pltpu.bitcast(weight_rows(j, m, q), u32)

    def prep_gu(m, j=None):
        st = min(RP, 128)
        for q in range(QC // 128):
            blocks = [s * QC // 128 + q for s in range(n)]
            if j is None:
                wt = [_from_words(wt_v[pl.ds((m * FC + 128 * b) // 2, 64), 0:D]) for b in blocks]
            else:
                wt = [weight_rows(j, m, b) for b in blocks]
            x = [[w[:, KB * k:KB * (k + 1)].astype(f32) for k in range(n)] for w in wt]
            where = [divmod(128 * q + r0, RP) for r0 in range(0, 128, st)]
            for i, a in enumerate(_lhs_terms(x)):
                for z, (p, r) in enumerate(where):
                    a_v[term(i, QC, KB, ((2 * p + m) * RP + r) // 2, st // 2)] = _to_words(a[z * st:(z + 1) * st])
            for s in range(n):
                for z, (p, r) in enumerate(where):
                    ar_v[pl.ds(((2 * (p * n + s) + m) * RP + r) // 2, st // 2), :] = pltpu.bitcast(
                        wt[s][z * st:(z + 1) * st, 512:D], u32)

    def prep_dn(j):
        x = [[wd_v[pl.ds(RD * a, RD), cols(j, b * KD, KD)].astype(f32) for b in range(nd)] for a in range(nd)]
        for i, a in enumerate(_lhs_terms(x)):
            ad_v[term(i, RD // 2, KD, 0, RD // 2)] = _to_words(a)

    def gate_up(t, p):
        sl = pl.ds(t * W, W)
        m = [None] * nm
        for g in (1, 3, 2, 4, 0, 5, 6):
            for i in range(g * nm // 7, (g + 1) * nm // 7):
                m[i] = _dot(_from_words(a_v[term(i, QC, KB, p * RP, RP)]),
                            _from_words(hb_v[pl.ds(i * KB // 2, KB // 2), sl]))
        ar = _from_words(ar_v[pl.ds(p * n * RP, n * RP), :])
        r = [_dot(ar, _from_words(hr_v[pl.ds(32 * s, 32), sl])) for s in range(n)]
        c = _assemble(m)
        c = [[c[a][b] + r[b][2 * a * RP:2 * (a + 1) * RP] for b in range(n)] for a in range(n)]
        hh = [[x[0:RP] * x[RP:2 * RP] for x in row] for row in c]
        k = n // nd
        for a in range(k):
            for b in range(k):
                sub = [[hh[x * k + a][y * k + b] for y in range(nd)] for x in range(nd)]
                for i, z in enumerate(_rhs_terms(sub)):
                    g_v[term((t % 2) * nmd + i, KD // 2, WD, (a * QC + p * RP) // 2, RP // 2, b * W, W)] = _to_words(z)

    def down_term(t, i, lo, size):
        return _dot(_from_words(ad_v[term(i, RD // 2, KD, 0, RD // 2)]),
                    _from_words(g_v[term((t % 2) * nmd + i, KD // 2, WD, 0, KD // 2, lo, size)]))

    def down(t, first=False):
        for i in range(nmd):
            at = pl.ds(i * RD, RD), pl.ds(t * WD, WD)
            y = down_term(t, i, 0, WD)
            acc_v[at] = y if first else acc_v[at] + y

    out_sem = sems.at[next(sem_i)]

    def down_last(t):
        per, half = nmd // 7, nd // 2
        for b in range(WD // W):
            part = {}

            def emit(qa, qb, c):
                for s in range(half):
                    for u in range(W // 128):
                        col = pl.ds(128 * (n * (t * W // 128 + u) + (qb * half + s) * (n // nd) + b), 128)
                        for a in range(half):
                            r0 = RD * (qa * half + a)
                            z = c[a][s][:, 128 * u:128 * (u + 1)]
                            out_v[pl.ds(r0, RD), col] = (
                                x1_v[pl.ds(r0, RD), col] + modc_v[pl.ds(5 * D + r0, RD), :] * z).astype(bf16)
                        rr = pl.ds(qa * D // 2, D // 2)
                        cp(out_v.at[rr, col], out_hbm.at[rr, col], out_sem).start()

            for g in (1, 3, 2, 4, 0, 6, 5):
                part[g] = _assemble([acc_v[pl.ds(i * RD, RD), pl.ds(t * WD + b * W, W)] + down_term(t, i, b * W, W)
                                     for i in range(g * per, (g + 1) * per)])
                if g == 3:
                    emit(1, 0, _add(part[1], part[3]))
                elif g == 4:
                    emit(0, 1, _add(part[2], part[4]))
                elif g == 6:
                    emit(0, 0, _add(_sub(_add(part[0], part[3]), part[4]), part[6]))
                elif g == 5:
                    emit(1, 1, _add(_add(_sub(part[0], part[1]), part[2]), part[5]))

    copies = {}
    for item in ORDER:
        op, arg = item[0], item[1:]
        if op == '|':
            pl.semaphore_signal(bar_sem, 1)
            pl.semaphore_wait(bar_sem, 1)
        elif op == 's':
            for name in arg.split('+'):
                copies[name] = make_copies(name)
                for d in copies[name]:
                    d.start(priority=1 if name in BULK else 0)
        elif op == 'w':
            with scope('w_' + arg):
                for name in arg.split('+'):
                    for d in copies[name]:
                        d.wait()
        elif op in 'qkv':
            proj('qkv'.index(op), int(arg))
        elif op == 'a':
            attn_col(2 * int(arg))
            attn_col(2 * int(arg) + 1)
        elif op == 'b':
            attn_col(int(arg))
        elif op == 'l':
            ln1(int(arg))
        elif op == 'S':
            ln1_stats(int(arg))
        elif op == 'N':
            ln1_apply(int(arg))
        elif op == 'o':
            wo(int(arg))
        elif op == 'n':
            ln2(int(arg))
        elif op == 'g':
            gate_up(int(arg[0]), int(arg[1]))
        elif op == 'd':
            down(int(arg), True)
        elif op == 'p':
            if arg in 'qkv':
                prep_qkv('qkv'.index(arg))
            elif arg == 'o':
                prep_wo()
            elif arg[0] == 'd':
                prep_dn(int(arg[1]))
            else:
                prep_gu('gu'.index(arg[0]))
        elif op == 't':
            transpose_gu(int(arg))
        elif op == 'z':
            acc_v[:, pl.ds((NFT - 1) * WD, WD)] = jnp.zeros((nmd * RD, WD), f32)
        elif op == 'm':
            mod_cols(*((0, 1152), (1152, 3456))[int(arg)])

    def chunk(j, last):
        down(NFT - 1)
        for t in range(NFT):
            if not (last and t == NFT - 1):
                for p in range(NP):
                    gate_up((t + 1) % NFT, p)
            if t == 0:
                prep_dn(j)
            if t == NFT - 2 and not last:
                prep_gu(0, j + 1)
                prep_gu(1, j + 1)
            if last:
                down_last(t)
            elif t < NFT - 1:
                down(t)

    if SHORT:
        def keep(j, carry):
            r = pl.ds(pl.multiple_of(j * 8, 8), 8)
            z = acc_v[r, 0:128]
            for ref in (a_v, ad_v, g_v, hb_v, hr_v):
                z = z + pltpu.bitcast(ref[r, 0:128], f32)
            z = z + x1_v[r, 0:128] + modc_v[r, :]
            z = z + jnp.tile(pltpu.bitcast(ar_v[r, :], f32), (1, 2))
            x1_v[r, 0:128] = z
            return carry
        lax.fori_loop(0, 4, keep, None)
        out_v[0:16, 0:128] = x1_v[0:16, 0:128].astype(bf16)
        d = cp(out_v, out_hbm, sems.at[next(sem_i)])
        d.start()
        d.wait()
        return
    trips = (NC - 2) // UN

    def body(i, carry):
        for u in range(UN):
            chunk(1 + UN * i + u, False)
        return carry

    with scope('loop'):
        lax.fori_loop(0, trips, body, None)
    for j in range(1 + UN * trips, NC - 1):
        chunk(j, False)
    chunk(NC - 1, True)
    with scope('w_out'):
        cp(out_v, out_hbm, out_sem).wait()


PRO = 'sc+q+m0+x00+x11+k+v+x24+x57+wo+m1+f00+f11+f28 z wq pq wc+m0 m0 wx00 l0 q0 wx11+k l1 q1 pk wv k0 k1 pv wx24 '
PLANS = {
    0: PRO + 'v0,v1,l2,l3,q2,k2,v2,a0,a1,q3,k3,v3,l4,a2,wx57+wo+m1+f00+f11,po,m1,t0,l5,q4,k4,v4,o0,o1,a3,n0,pg,pu,o2,o3,l6,q5,k5,v5,G0,a4,n1,l7,q6,k6,v6,G1,a5,pd0,o4,q7,k7,v7,a6,o5,n2,D0,G2,a7,t1,o6,o7,D1,n3,G3,pg,pu,D2,G0,wf28'.replace(',', ' '),
    1: PRO.replace('+f28', '') + 'v0,v1,l2,l3,q2,k2,v2,a0,a1,q3,k3,v3,l4,a2,wx57+wo+m1+f00+f11,sf28,po,m1,t0,l5,q4,k4,v4,o0,o1,a3,n0,pg,pu,o2,o3,l6,q5,k5,v5,G0,a4,n1,l7,q6,k6,v6,G1,a5,pd0,o4,q7,k7,v7,a6,o5,n2,D0,G2,a7,t1,o6,o7,D1,n3,G3,pg,pu,D2,G0,wf28'.replace(',', ' '),
}


def make(L=1, LD=1, NP=1, scopes=False, plan=0, ev=True, short=False, SL=16, UN=1, BULK=()):
    ORDER = []
    for item in (PLANS[plan] if isinstance(plan, int) else PRO + plan.replace(',', ' ')).split():
        if item[0] == 'G':
            ORDER += ['g%s%d' % (item[1], p) for p in range(NP)]
        elif item[0] == 'D':
            ORDER += [] if item[-1] == 'X' else ['d' + item[1]]
        else:
            ORDER.append(item)
    flags = {'XLA_TPU_EVENLY_DISTRIBUTE_CRITICAL_NODES': True} if ev else {}
    n, nm, nd, nmd = 2 ** L, 7 ** L, 2 ** LD, 7 ** LD

    def terms(count, per, width):
        return ((count + 1) // 2 * per, 256) if width == 128 else (count * per, width)

    @jax.jit
    def f(A_x, A_wqkv, A_wo, B_x, B_w_gate, B_w_up, B_w_down, c, w_mod):
        xT = A_x[0].T
        wdT = B_w_down.T
        hbm = pl.BlockSpec(memory_space=pltpu.HBM)
        V = pltpu.VMEM
        outT = pl.pallas_call(
            functools.partial(kernel, L=L, LD=LD, NP=NP, scopes=scopes, ORDER=ORDER, SHORT=short, SL=SL, UN=UN, BULK=BULK),
            in_specs=[hbm] * 8,
            out_specs=hbm,
            out_shape=jax.ShapeDtypeStruct((D, S), bf16),
            scratch_shapes=[
                V((1, D), bf16), V((D, 6 * D), bf16), V((D, S), bf16), V((D, 3 * D), bf16), V((D, D), bf16),
                V((5, 3 * D, 128), f32), V((3 * D // 2, 640), u32), V((D // 2, 640), u32), V((6 * D, 128), f32),
                V((D // 2, S), u32), V((D // 2, S), u32), V((D // 2, S + 128), u32), V((D // 2, S + 128), u32),
                V((D // 2, S), u32), V((D, S), f32), V((32, S), f32), V((nm * 256 // n, S // n), u32), V((n * 32, S // n), u32),
                V((D, F), bf16), V((D, F), bf16), V((D, F), bf16), V((FC, 640), u32),
                V(terms(nm, FC // n, 512 // n), u32), V((FC, 64), u32), V(terms(nmd, D // nd // 2, FC // nd), u32),
                V(terms(2 * nmd, FC // nd // 2, 512 // nd), u32), V((nmd * D // nd, S // nd), f32), V((D, S), bf16),
                pltpu.SemaphoreType.DMA((64,)), pltpu.SemaphoreType.REGULAR,
            ],
            compiler_params=pltpu.CompilerParams(flags=flags, vmem_limit_bytes=120 * 1024 * 1024),
        )(xT, A_wqkv, A_wo, B_w_gate, B_w_up, wdT, c, w_mod)
        return outT.T[None]
    return f


pallas_adaLN_cond__sliding_local_dilated__glu_gated_bilinear__prompt_kernel = make(L=2, LD=2, NP=4)
```

```python
import functools

import jax
import jax.numpy as jnp
from jax import lax
import jax.experimental.pallas as pl
import jax.experimental.pallas.tpu as pltpu

D, H, DH, F, S = 576, 32, 18, 4608, 2048
WIN, DIL = 8, 2
EPS = 1e-5
TN = 256
FN = 512
FC = 512
NB = 4
TERMS = 49
KS = 512
RD = D // NB
RP = 32

f32, bf16, u32 = jnp.float32, jnp.bfloat16, jnp.uint32


def _dot(a, b):
    return jnp.dot(a, b, preferred_element_type=f32)


def _to_words(x):
    return pltpu.bitcast(x.astype(bf16), u32)


def _from_words(x):
    return pltpu.bitcast(x, bf16)


def _halves(x):
    return tuple(pltpu.unpack_elementwise(x, index=i, packed_dtype=bf16, unpacked_dtype=f32) for i in range(2))


def _add(x, y):
    return [[a + b for a, b in zip(r, s)] for r, s in zip(x, y)]


def _sub(x, y):
    return [[a - b for a, b in zip(r, s)] for r, s in zip(x, y)]


def _quadrants(x):
    h = len(x) // 2
    return [r[:h] for r in x[:h]], [r[h:] for r in x[:h]], [r[:h] for r in x[h:]], [r[h:] for r in x[h:]]


def _lhs_terms(x):
    if len(x) == 1:
        return [x[0][0]]
    a11, a12, a21, a22 = _quadrants(x)
    terms = (_add(a11, a22), _add(a21, a22), a11, a22, _add(a11, a12), _sub(a21, a11), _sub(a12, a22))
    return [z for y in terms for z in _lhs_terms(y)]


def _rhs_terms(x):
    if len(x) == 1:
        return [x[0][0]]
    b11, b12, b21, b22 = _quadrants(x)
    terms = (_add(b11, b22), b11, _sub(b12, b22), _sub(b21, b11), b22, _add(b11, b12), _add(b21, b22))
    return [z for y in terms for z in _rhs_terms(y)]


def _quadrant(a, b, p):
    if (a, b) == (0, 0):
        return _add(_sub(_add(p[0], p[3]), p[4]), p[6])
    if (a, b) == (0, 1):
        return _add(p[2], p[4])
    if (a, b) == (1, 0):
        return _add(p[1], p[3])
    return _add(_add(_sub(p[0], p[1]), p[2]), p[5])


def _assemble(m):
    if len(m) == 1:
        return [[m[0]]]
    n = len(m) // 7
    p = [_assemble(m[i * n:(i + 1) * n]) for i in range(7)]
    c = [[_quadrant(a, b, p) for b in range(2)] for a in range(2)]
    return [x + y for x, y in zip(*c[0])] + [x + y for x, y in zip(*c[1])]


def _term(i, rows, r0, nr):
    return pl.ds((i // 2) * rows + r0, nr), pl.ds((i % 2) * 128, 128)


def _col_mean(x):
    r = x.shape[0] // 4
    return jnp.sum((x[0:r] + x[r:2 * r]) + (x[2 * r:3 * r] + x[3 * r:]), axis=0, keepdims=True) * (1.0 / D)


def _kernel(x_hbm, wqkv_hbm, wo_hbm, wg_hbm, wu_hbm, wd_hbm, c_hbm, wmod_hbm, out_hbm,
            c_v, wmod_v, x_v, wqkv_v, wo_v, tmp_v, wqkvT_v, woT_v, mod_v,
            h_v, q_v, k_v, v_v, o_v, x1_v, stat_v, hb_v, hr_v,
            wg_v, wu_v, wd_v, wt_v, a_v, ar_v, ad_v, g_v, acc_v, out_v, sems):
    sem_ids = iter(range(sems.shape[0]))
    out_sem = sems.at[next(sem_ids)]

    def fetch(src, dst, lo=None, hi=None):
        if lo is not None:
            src, dst = src.at[:, pl.ds(lo, hi - lo)], dst.at[:, pl.ds(lo, hi - lo)]
        copy = pltpu.make_async_copy(src, dst, sems.at[next(sem_ids)])
        copy.start()
        return [copy]

    def fetch_glu(j0, j1):
        return sum((fetch(s, d, j0 * FC, j1 * FC) for s, d in ((wg_hbm, wg_v), (wu_hbm, wu_v), (wd_hbm, wd_v))), [])

    def wait(*groups):
        for group in groups:
            for copy in group:
                copy.wait()

    def modulation(lo, hi):
        c = c_v[...].astype(f32)
        act = jnp.broadcast_to(c * jax.nn.sigmoid(c), (16, D)).astype(bf16)
        m = _dot(act, wmod_v[:, pl.ds(lo, hi - lo)])[0:8]
        idx = lo + lax.broadcasted_iota(jnp.int32, m.shape, 1)
        is_scale = ((idx >= D) & (idx < 2 * D)) | ((idx >= 4 * D) & (idx < 5 * D))
        m = m + jnp.where(is_scale, 1.0, 0.0)
        for j in range((hi - lo) // 128):
            mod_v[pl.ds(lo + 128 * j, 128), :] = jnp.tile(m[:, 128 * j:128 * (j + 1)], (16, 1)).T

    SHIFT_A, SCALE_A, GATE_A, SHIFT_B, SCALE_B, GATE_B = range(6)

    def mod(i, r0=0, nr=D):
        return mod_v[pl.ds(i * D + r0, nr), :]

    def norm_a(t):
        for j in range(2 * t, 2 * t + 2):
            c = pl.ds(128 * j, 128)
            x = x_v[:, c].astype(f32)
            xc = x - _col_mean(x)
            h_v[:, c] = _to_words(xc * lax.rsqrt(_col_mean(xc * xc) + EPS) * mod(SCALE_A) + mod(SHIFT_A))

    def prepare_qkv(p):
        for kb in range(5):
            kw = min(128, D - 128 * kb)
            for j in (range(0, 5), range(5, 9), range(9, 14))[p]:
                w = min(128, 3 * D - 128 * j)
                blk = wqkv_v[pl.ds(128 * kb, kw), pl.ds(128 * j, w)].astype(f32)
                if w < 128:
                    blk = jnp.concatenate([blk, jnp.zeros((kw, 128 - w), f32)], axis=1)
                if kw < 128:
                    blk = jnp.concatenate([blk, jnp.zeros((128 - kw, 128), f32)], axis=0)
                tmp_v[kb, pl.ds(128 * j, w), :] = blk.T[0:w]
            for d in range(DH):
                rows = tmp_v[kb, pl.ds(p * D + d, H, stride=DH), :]
                wqkvT_v[pl.ds((p * D + d * H) // 2, H // 2), pl.ds(128 * kb, 128)] = _to_words(rows)

    def prepare_out():
        for nb in range(5):
            nw = min(128, D - 128 * nb)
            blk = wo_v[:, pl.ds(128 * nb, nw)].astype(f32)
            if nw < 128:
                blk = jnp.concatenate([blk, jnp.zeros((D, 128 - nw), f32)], axis=1)
            tmp_v[nb, pl.ds(0, D), :] = blk
            for eb in range(5):
                rows = [tmp_v[nb, pl.ds(d, H, stride=DH), :] for d in range(4 * eb, min(4 * eb + 4, DH))]
                if len(rows) < 4:
                    rows.append(jnp.zeros((128 - H * len(rows), 128), f32))
                woT_v[pl.ds(64 * nb, nw // 2), pl.ds(128 * eb, 128)] = _to_words(
                    jnp.concatenate(rows, axis=0).T[0:nw])

    def project(p, t):
        w = _from_words(wqkvT_v[pl.ds(p * D // 2, D // 2), :])[:, 0:D]
        y = _to_words(_dot(w, _from_words(h_v[:, pl.ds(t * TN, TN)])))
        if p == 0:
            q_v[:, pl.ds(t * TN, TN)] = y
        else:
            ref = (k_v, v_v)[p - 1]
            ref[:, pl.ds(128 + t * TN, TN)] = y
            if t == 0:
                ref[:, pl.ds(0, 128)] = jnp.broadcast_to(y[:, 0:1], (D // 2, 128))

    def project_all(t):
        for p in range(3):
            project(p, t)

    lane = lax.broadcasted_iota(jnp.int32, (8, 128), 1)

    def window(ref, r, j):
        cur = ref[pl.ds(r, 8), pl.ds(128 * (j + 1), 128)]
        prev = ref[pl.ds(r, 8), pl.ds(128 * j, 128)]
        yield _halves(cur)
        for w in range(1, WIN):
            yield _halves(pltpu.roll(jnp.where(lane < 128 - DIL * w, cur, prev), DIL * w, 1))

    def attend(t):
        for j in range(2 * t, 2 * t + 2):
            c = pl.ds(128 * j, 128)
            for hg in range(2):
                logits = [[None] * WIN, [None] * WIN]
                for d in range(DH):
                    r = d * (H // 2) + hg * 8
                    q = _halves(q_v[pl.ds(r, 8), c])
                    for w, k in enumerate(window(k_v, r, j)):
                        for s in range(2):
                            qk = q[s] * k[s]
                            logits[s][w] = qk if d == 0 else logits[s][w] + qk
                probs = []
                for s in range(2):
                    z = [x * DH ** -0.5 for x in logits[s]]
                    if j == 0:
                        z = [x if w == 0 else jnp.where(lane >= DIL * w, x, -1e9) for w, x in enumerate(z)]
                    top = functools.reduce(jnp.maximum, z)
                    e = [jnp.exp(x - top) for x in z]
                    inv = 1.0 / functools.reduce(jnp.add, e)
                    probs.append([x * inv for x in e])
                for d in range(DH):
                    r = d * (H // 2) + hg * 8
                    o = [None, None]
                    for w, v in enumerate(window(v_v, r, j)):
                        for s in range(2):
                            pv = probs[s][w] * v[s]
                            o[s] = pv if w == 0 else o[s] + pv
                    o_v[pl.ds(r, 8), c] = pltpu.pack_elementwise(o, packed_dtype=bf16)

    def attention_out(t):
        y = _dot(_from_words(woT_v[...])[:, 0:D], _from_words(o_v[:, pl.ds(t * TN, TN)]))
        for s in range(2):
            c = pl.ds(t * TN + 128 * s, 128)
            x1 = x_v[:, c].astype(f32) + mod(GATE_A) * y[:, 128 * s:128 * (s + 1)]
            x1_v[:, c] = x1
            dev = x1 - x1[0:1]
            m = jnp.sum(dev, axis=0, keepdims=True) * (1.0 / D)
            var = jnp.sum(dev * dev, axis=0, keepdims=True) * (1.0 / D) - m * m
            stat_v[0:8, c] = jnp.broadcast_to(m + x1[0:1], (8, 128))
            stat_v[8:16, c] = jnp.broadcast_to(var, (8, 128))

    def norm_b(t):
        cs = [pl.ds(t * FN + 128 * s, 128) for s in range(NB)]
        mean = [stat_v[0:1, c] for c in cs]
        rstd = [lax.rsqrt(jnp.maximum(stat_v[8:9, c], 0.0) + EPS) for c in cs]

        def h(r0, nr, s):
            return (x1_v[pl.ds(r0, nr), cs[s]] - mean[s]) * rstd[s] * mod(SCALE_B, r0, nr) + mod(SHIFT_B, r0, nr)

        c = pl.ds(128 * t, 128)
        for r0 in range(0, 128, 16):
            for i, b in enumerate(_rhs_terms([[h(128 * k + r0, 16, s) for s in range(NB)] for k in range(NB)])):
                hb_v[pl.ds((128 * i + r0) // 2, 8), c] = _to_words(b)
        for s in range(NB):
            hr_v[pl.ds(32 * s, 32), c] = _to_words(h(KS, D - KS, s))

    def chunk_cols(j, b):
        start = j * FC + 128 * b
        return pl.ds(start if isinstance(start, int) else pl.multiple_of(start, 128), 128)

    def weight_rows(j, m, b):
        return (wg_v, wu_v)[m][:, chunk_cols(j, b)].T

    def stage_gate_up(j):
        for m in range(2):
            for b in range(NB):
                wt_v[pl.ds((m * FC + 128 * b) // 2, 64), 0:D] = pltpu.bitcast(weight_rows(j, m, b), u32)

    def prepare_gate_up(j=None):
        for m in range(2):
            if j is None:
                wt = [_from_words(wt_v[pl.ds((m * FC + 128 * b) // 2, 64), 0:D]) for b in range(NB)]
            else:
                wt = [weight_rows(j, m, b) for b in range(NB)]
            blocks = [[w[:, 128 * k:128 * (k + 1)].astype(f32) for k in range(NB)] for w in wt]
            for i, a in enumerate(_lhs_terms(blocks)):
                for p in range(128 // RP):
                    a_v[_term(i, 128, (2 * p + m) * RP // 2, RP // 2)] = _to_words(a[p * RP:(p + 1) * RP])
            for b in range(NB):
                for p in range(128 // RP):
                    ar_v[pl.ds((2 * (p * NB + b) + m) * RP // 2, RP // 2), :] = pltpu.bitcast(
                        wt[b][p * RP:(p + 1) * RP, KS:D], u32)

    def prepare_down(j):
        blocks = [[wd_v[pl.ds(RD * a, RD), chunk_cols(j, b)].astype(f32) for b in range(NB)] for a in range(NB)]
        for i, a in enumerate(_lhs_terms(blocks)):
            ad_v[_term(i, RD // 2, 0, RD // 2)] = _to_words(a)

    def gate_up(t):
        c = pl.ds(128 * t, 128)
        for p in range(128 // RP):
            prod = [None] * TERMS
            for g in (1, 3, 2, 4, 0, 5, 6):
                for i in range(7 * g, 7 * g + 7):
                    prod[i] = _dot(_from_words(a_v[_term(i, 128, p * RP, RP)]), _from_words(hb_v[pl.ds(64 * i, 64), c]))
            rest_w = _from_words(ar_v[pl.ds(p * NB * RP, NB * RP), :])
            rest = [_dot(rest_w, _from_words(hr_v[pl.ds(32 * s, 32), c])) for s in range(NB)]
            gu = _assemble(prod)
            gu = [[gu[a][b] + rest[b][2 * a * RP:2 * (a + 1) * RP] for b in range(NB)] for a in range(NB)]
            hidden = [[x[0:RP] * x[RP:2 * RP] for x in row] for row in gu]
            for i, z in enumerate(_rhs_terms(hidden)):
                g_v[_term((t % 2) * TERMS + i, 64, p * RP // 2, RP // 2)] = _to_words(z)

    def down_product(t, i):
        return _dot(_from_words(ad_v[_term(i, RD // 2, 0, RD // 2)]),
                    _from_words(g_v[_term((t % 2) * TERMS + i, 64, 0, 64)]))

    def down(t, first=False):
        for i in range(TERMS):
            at = pl.ds(i * RD, RD), pl.ds(128 * t, 128)
            y = down_product(t, i)
            acc_v[at] = y if first else acc_v[at] + y

    def down_and_write(t):
        part = {}
        for g, done in ((1, None), (3, (1, 0)), (2, None), (4, (0, 1)), (0, None), (6, (0, 0)), (5, (1, 1))):
            part[g] = _assemble([acc_v[pl.ds(i * RD, RD), pl.ds(128 * t, 128)] + down_product(t, i)
                                 for i in range(7 * g, 7 * g + 7)])
            if done is None:
                continue
            y = _quadrant(*done, part)
            for s in range(2):
                c = pl.ds(t * FN + 128 * (2 * done[1] + s), 128)
                for a in range(2):
                    r0 = RD * (2 * done[0] + a)
                    out_v[pl.ds(r0, RD), c] = (x1_v[pl.ds(r0, RD), c] + mod(GATE_B, r0, RD) * y[a][s]).astype(bf16)
                rows = pl.ds(done[0] * D // 2, D // 2)
                pltpu.make_async_copy(out_v.at[rows, c], out_hbm.at[rows, c], out_sem).start()

    def glu_chunk(j, last):
        finish = down_and_write if last else down
        down(3)
        gate_up(1)
        prepare_down(j)
        finish(0)
        gate_up(2)
        finish(1)
        gate_up(3)
        if not last:
            prepare_gate_up(j + 1)
        finish(2)
        if last:
            finish(3)
        else:
            gate_up(0)

    got_c = fetch(c_hbm, c_v)
    got_q = fetch(wqkv_hbm, wqkv_v, 0, 640)
    got_mod_a = fetch(wmod_hbm, wmod_v, 0, 2 * D)
    got_x0 = fetch(x_hbm, x_v, 0, TN)
    got_x1 = fetch(x_hbm, x_v, TN, 2 * TN)
    got_k = fetch(wqkv_hbm, wqkv_v, 640, 1152)
    got_v = fetch(wqkv_hbm, wqkv_v, 1152, 3 * D)
    got_x2 = fetch(x_hbm, x_v, 2 * TN, 5 * TN)
    got_x5 = fetch(x_hbm, x_v, 5 * TN, S)
    got_wo = fetch(wo_hbm, wo_v)
    got_mod_b = fetch(wmod_hbm, wmod_v, 2 * D, 6 * D)
    got_glu0 = fetch_glu(0, 1)
    got_glu1 = fetch_glu(1, 2)
    got_glu2 = fetch_glu(2, F // FC)

    acc_v[:, pl.ds(3 * 128, 128)] = jnp.zeros((TERMS * RD, 128), f32)
    wait(got_q)
    prepare_qkv(0)
    wait(got_c, got_mod_a)
    modulation(0, 2 * D)
    wait(got_x0)
    norm_a(0); project(0, 0)
    wait(got_x1, got_k)
    norm_a(1); project(0, 1); prepare_qkv(1)
    wait(got_v)
    project(1, 0); project(1, 1); prepare_qkv(2)
    wait(got_x2)
    project(2, 0); project(2, 1); norm_a(2); norm_a(3)
    project_all(2); attend(0); attend(1)
    project_all(3); norm_a(4); attend(2)
    wait(got_x5, got_wo, got_mod_b, got_glu0, got_glu1)
    prepare_out(); modulation(2 * D, 6 * D); stage_gate_up(0); norm_a(5)
    project_all(4); attention_out(0); attention_out(1); attend(3); norm_b(0); prepare_gate_up()
    attention_out(2); attention_out(3); norm_a(6)
    project_all(5); gate_up(0); attend(4); norm_b(1); norm_a(7)
    project_all(6); gate_up(1); attend(5); prepare_down(0); attention_out(4)
    project_all(7); attend(6); attention_out(5); norm_b(2); down(0, first=True)
    gate_up(2); attend(7); stage_gate_up(1); attention_out(6); attention_out(7); down(1, first=True)
    norm_b(3); gate_up(3); prepare_gate_up(); down(2, first=True); gate_up(0)
    wait(got_glu2)
    lax.fori_loop(1, F // FC - 1, lambda j, carry: glu_chunk(j, False), None)
    glu_chunk(F // FC - 1, True)
    pltpu.make_async_copy(out_v, out_hbm, out_sem).wait()


@jax.jit
def pallas_adaLN_cond__sliding_local_dilated__glu_gated_bilinear__prompt_kernel(
    A_x: jax.Array,
    A_wqkv: jax.Array,
    A_wo: jax.Array,
    B_x: jax.Array,
    B_w_gate: jax.Array,
    B_w_up: jax.Array,
    B_w_down: jax.Array,
    c: jax.Array,
    w_mod: jax.Array,
):
    del B_x
    hbm = pl.BlockSpec(memory_space=pltpu.HBM)
    vmem = pltpu.VMEM
    pairs = (TERMS + 1) // 2
    out = pl.pallas_call(
        _kernel,
        in_specs=[hbm] * 8,
        out_specs=hbm,
        out_shape=jax.ShapeDtypeStruct((D, S), bf16),
        scratch_shapes=[
            vmem((1, D), bf16), vmem((D, 6 * D), bf16), vmem((D, S), bf16),
            vmem((D, 3 * D), bf16), vmem((D, D), bf16), vmem((5, 3 * D, 128), f32),
            vmem((3 * D // 2, 640), u32), vmem((D // 2, 640), u32),
            vmem((6 * D, 128), f32),
            vmem((D // 2, S), u32), vmem((D // 2, S), u32),
            vmem((D // 2, S + 128), u32), vmem((D // 2, S + 128), u32),
            vmem((D // 2, S), u32), vmem((D, S), f32), vmem((16, S), f32),
            vmem((TERMS * 64, S // NB), u32), vmem((NB * 32, S // NB), u32),
            vmem((D, F), bf16), vmem((D, F), bf16), vmem((D, F), bf16),
            vmem((FC, 640), u32),
            vmem((pairs * 128, 256), u32), vmem((FC, D - KS), u32),
            vmem((pairs * RD // 2, 256), u32),
            vmem((TERMS * 64, 256), u32),
            vmem((TERMS * RD, S // NB), f32), vmem((D, S), bf16),
            pltpu.SemaphoreType.DMA((24,)),
        ],
        compiler_params=pltpu.CompilerParams(
            flags={"XLA_TPU_EVENLY_DISTRIBUTE_CRITICAL_NODES": True},
            vmem_limit_bytes=120 * 1024 * 1024),
    )(A_x[0].T, A_wqkv, A_wo, B_w_gate, B_w_up, B_w_down.T, c, w_mod)
    return out.T[None]
```

```python
import functools

import jax
import jax.numpy as jnp
from jax import lax
import jax.experimental.pallas as pl
import jax.experimental.pallas.tpu as pltpu

D, H, DH, F, S = 576, 32, 18, 4608, 2048
WIN, DIL = 8, 2
EPS = 1e-5
TN = 256
FN = 512
FC = 512
NB = 4
TERMS = 49
TERM_ORDER = [7 * g + i for g in (1, 3, 2, 4, 0, 5, 6) for i in range(7)]
KS = 512
RD = D // NB
RP = 32

f32, bf16, u32 = jnp.float32, jnp.bfloat16, jnp.uint32


def _dot(a, b):
    return jnp.dot(a, b, preferred_element_type=f32)


def _to_words(x):
    return pltpu.bitcast(x.astype(bf16), u32)


def _from_words(x):
    return pltpu.bitcast(x, bf16)


def _halves(x):
    return tuple(pltpu.unpack_elementwise(x, index=i, packed_dtype=bf16, unpacked_dtype=f32) for i in range(2))


def _add(x, y):
    return [[a + b for a, b in zip(r, s)] for r, s in zip(x, y)]


def _sub(x, y):
    return [[a - b for a, b in zip(r, s)] for r, s in zip(x, y)]


def _quadrants(x):
    h = len(x) // 2
    return [r[:h] for r in x[:h]], [r[h:] for r in x[:h]], [r[:h] for r in x[h:]], [r[h:] for r in x[h:]]


def _lhs_terms(x):
    if len(x) == 1:
        return [x[0][0]]
    a11, a12, a21, a22 = _quadrants(x)
    terms = (_add(a11, a22), _add(a21, a22), a11, a22, _add(a11, a12), _sub(a21, a11), _sub(a12, a22))
    return [z for y in terms for z in _lhs_terms(y)]


def _rhs_terms(x):
    if len(x) == 1:
        return [x[0][0]]
    b11, b12, b21, b22 = _quadrants(x)
    terms = (_add(b11, b22), b11, _sub(b12, b22), _sub(b21, b11), b22, _add(b11, b12), _add(b21, b22))
    return [z for y in terms for z in _rhs_terms(y)]


def _quadrant(a, b, p):
    if (a, b) == (0, 0):
        return _add(_sub(_add(p[0], p[3]), p[4]), p[6])
    if (a, b) == (0, 1):
        return _add(p[2], p[4])
    if (a, b) == (1, 0):
        return _add(p[1], p[3])
    return _add(_add(_sub(p[0], p[1]), p[2]), p[5])


def _assemble(m):
    if len(m) == 1:
        return [[m[0]]]
    n = len(m) // 7
    p = [_assemble(m[i * n:(i + 1) * n]) for i in range(7)]
    c = [[_quadrant(a, b, p) for b in range(2)] for a in range(2)]
    return [x + y for x, y in zip(*c[0])] + [x + y for x, y in zip(*c[1])]


def _term(i, rows, r0, nr):
    return pl.ds((i // 2) * rows + r0, nr), pl.ds((i % 2) * 128, 128)


def _col_mean(x):
    r = x.shape[0] // 4
    return jnp.sum((x[0:r] + x[r:2 * r]) + (x[2 * r:3 * r] + x[3 * r:]), axis=0, keepdims=True) * (1.0 / D)


def _kernel(x_hbm, wqkv_hbm, wo_hbm, wg_hbm, wu_hbm, wd_hbm, c_hbm, wmod_hbm, out_hbm,
            c_v, wmod_v, x_v, wqkv_v, wo_v, tmp_v, wqkvT_v, woT_v, mod_v,
            h_v, q_v, k_v, v_v, o_v, x1_v, stat_v, hb_v, hr_v,
            wg_v, wu_v, wd_v, wt_v, a_v, ar_v, ad_v, g_v, acc_v, out_v, sems):
    sem_ids = iter(range(sems.shape[0]))
    out_sem = sems.at[next(sem_ids)]

    def fetch(src, dst, lo=None, hi=None):
        if lo is not None:
            src, dst = src.at[:, pl.ds(lo, hi - lo)], dst.at[:, pl.ds(lo, hi - lo)]
        copy = pltpu.make_async_copy(src, dst, sems.at[next(sem_ids)])
        copy.start()
        return [copy]

    def fetch_glu(j0, j1):
        return sum((fetch(s, d, j0 * FC, j1 * FC) for s, d in ((wg_hbm, wg_v), (wu_hbm, wu_v), (wd_hbm, wd_v))), [])

    def wait(*groups):
        for group in groups:
            for copy in group:
                copy.wait()

    def modulation(lo, hi):
        c = c_v[...].astype(f32)
        act = jnp.broadcast_to(c * jax.nn.sigmoid(c), (16, D)).astype(bf16)
        m = _dot(act, wmod_v[:, pl.ds(lo, hi - lo)])[0:8]
        idx = lo + lax.broadcasted_iota(jnp.int32, m.shape, 1)
        is_scale = ((idx >= D) & (idx < 2 * D)) | ((idx >= 4 * D) & (idx < 5 * D))
        m = m + jnp.where(is_scale, 1.0, 0.0)
        for j in range((hi - lo) // 128):
            mod_v[pl.ds(lo + 128 * j, 128), :] = jnp.tile(m[:, 128 * j:128 * (j + 1)], (16, 1)).T

    SHIFT_A, SCALE_A, GATE_A, SHIFT_B, SCALE_B, GATE_B = range(6)

    def mod(i, r0=0, nr=D):
        return mod_v[pl.ds(i * D + r0, nr), :]

    def norm_a(t):
        for j in range(2 * t, 2 * t + 2):
            c = pl.ds(128 * j, 128)
            x = x_v[:, c].astype(f32)
            xc = x - _col_mean(x)
            h_v[:, c] = _to_words(xc * lax.rsqrt(_col_mean(xc * xc) + EPS) * mod(SCALE_A) + mod(SHIFT_A))

    def prepare_qkv(p):
        for kb in range(5):
            kw = min(128, D - 128 * kb)
            for j in (range(0, 5), range(5, 9), range(9, 14))[p]:
                w = min(128, 3 * D - 128 * j)
                blk = wqkv_v[pl.ds(128 * kb, kw), pl.ds(128 * j, w)].astype(f32)
                if w < 128:
                    blk = jnp.concatenate([blk, jnp.zeros((kw, 128 - w), f32)], axis=1)
                if kw < 128:
                    blk = jnp.concatenate([blk, jnp.zeros((128 - kw, 128), f32)], axis=0)
                tmp_v[kb, pl.ds(128 * j, w), :] = blk.T[0:w]
            for d in range(DH):
                rows = tmp_v[kb, pl.ds(p * D + d, H, stride=DH), :]
                wqkvT_v[pl.ds((p * D + d * H) // 2, H // 2), pl.ds(128 * kb, 128)] = _to_words(rows)

    def prepare_out():
        for nb in range(5):
            nw = min(128, D - 128 * nb)
            blk = wo_v[:, pl.ds(128 * nb, nw)].astype(f32)
            if nw < 128:
                blk = jnp.concatenate([blk, jnp.zeros((D, 128 - nw), f32)], axis=1)
            tmp_v[nb, pl.ds(0, D), :] = blk
            for eb in range(5):
                rows = [tmp_v[nb, pl.ds(d, H, stride=DH), :] for d in range(4 * eb, min(4 * eb + 4, DH))]
                if len(rows) < 4:
                    rows.append(jnp.zeros((128 - H * len(rows), 128), f32))
                woT_v[pl.ds(64 * nb, nw // 2), pl.ds(128 * eb, 128)] = _to_words(
                    jnp.concatenate(rows, axis=0).T[0:nw])

    def project(p, t):
        w = _from_words(wqkvT_v[pl.ds(p * D // 2, D // 2), :])[:, 0:D]
        y = _to_words(_dot(w, _from_words(h_v[:, pl.ds(t * TN, TN)])))
        if p == 0:
            q_v[:, pl.ds(t * TN, TN)] = y
        else:
            ref = (k_v, v_v)[p - 1]
            ref[:, pl.ds(128 + t * TN, TN)] = y
            if t == 0:
                ref[:, pl.ds(0, 128)] = jnp.broadcast_to(y[:, 0:1], (D // 2, 128))

    def project_all(t):
        for p in range(3):
            project(p, t)

    lane = lax.broadcasted_iota(jnp.int32, (8, 128), 1)

    def window(ref, r, j):
        cur = ref[pl.ds(r, 8), pl.ds(128 * (j + 1), 128)]
        prev = ref[pl.ds(r, 8), pl.ds(128 * j, 128)]
        yield _halves(cur)
        for w in range(1, WIN):
            yield _halves(pltpu.roll(jnp.where(lane < 128 - DIL * w, cur, prev), DIL * w, 1))

    def attend(t):
        for j in range(2 * t, 2 * t + 2):
            c = pl.ds(128 * j, 128)
            for hg in range(2):
                logits = [[None] * WIN, [None] * WIN]
                for d in range(DH):
                    r = d * (H // 2) + hg * 8
                    q = _halves(q_v[pl.ds(r, 8), c])
                    for w, k in enumerate(window(k_v, r, j)):
                        for s in range(2):
                            qk = q[s] * k[s]
                            logits[s][w] = qk if d == 0 else logits[s][w] + qk
                probs = []
                for s in range(2):
                    z = [x * DH ** -0.5 for x in logits[s]]
                    if j == 0:
                        z = [x if w == 0 else jnp.where(lane >= DIL * w, x, -1e9) for w, x in enumerate(z)]
                    top = functools.reduce(jnp.maximum, z)
                    e = [jnp.exp(x - top) for x in z]
                    inv = 1.0 / functools.reduce(jnp.add, e)
                    probs.append([x * inv for x in e])
                for d in range(DH):
                    r = d * (H // 2) + hg * 8
                    o = [None, None]
                    for w, v in enumerate(window(v_v, r, j)):
                        for s in range(2):
                            pv = probs[s][w] * v[s]
                            o[s] = pv if w == 0 else o[s] + pv
                    o_v[pl.ds(r, 8), c] = pltpu.pack_elementwise(o, packed_dtype=bf16)

    def attention_out(t):
        y = _dot(_from_words(woT_v[...])[:, 0:D], _from_words(o_v[:, pl.ds(t * TN, TN)]))
        for s in range(2):
            c = pl.ds(t * TN + 128 * s, 128)
            x1 = x_v[:, c].astype(f32) + mod(GATE_A) * y[:, 128 * s:128 * (s + 1)]
            x1_v[:, c] = x1
            dev = x1 - x1[0:1]
            m = jnp.sum(dev, axis=0, keepdims=True) * (1.0 / D)
            var = jnp.sum(dev * dev, axis=0, keepdims=True) * (1.0 / D) - m * m
            stat_v[0:8, c] = jnp.broadcast_to(m + x1[0:1], (8, 128))
            stat_v[8:16, c] = jnp.broadcast_to(var, (8, 128))

    def norm_b(t):
        cs = [pl.ds(t * FN + 128 * s, 128) for s in range(NB)]
        mean = [stat_v[0:1, c] for c in cs]
        rstd = [lax.rsqrt(jnp.maximum(stat_v[8:9, c], 0.0) + EPS) for c in cs]

        def h(r0, nr, s):
            return (x1_v[pl.ds(r0, nr), cs[s]] - mean[s]) * rstd[s] * mod(SCALE_B, r0, nr) + mod(SHIFT_B, r0, nr)

        c = pl.ds(128 * t, 128)
        for r0 in range(0, 128, 16):
            for i, b in enumerate(_rhs_terms([[h(128 * k + r0, 16, s) for s in range(NB)] for k in range(NB)])):
                hb_v[pl.ds((128 * i + r0) // 2, 8), c] = _to_words(b)
        for s in range(NB):
            hr_v[pl.ds(32 * s, 32), c] = _to_words(h(KS, D - KS, s))

    def chunk_cols(j, b):
        start = j * FC + 128 * b
        return pl.ds(start if isinstance(start, int) else pl.multiple_of(start, 128), 128)

    def weight_rows(j, m, b):
        return (wg_v, wu_v)[m][:, chunk_cols(j, b)].T

    def stage_gate_up(j):
        for m in range(2):
            for b in range(NB):
                wt_v[pl.ds((m * FC + 128 * b) // 2, 64), 0:D] = pltpu.bitcast(weight_rows(j, m, b), u32)

    def prepare_gate_up(j=None):
        for m in range(2):
            if j is None:
                wt = [_from_words(wt_v[pl.ds((m * FC + 128 * b) // 2, 64), 0:D]) for b in range(NB)]
            else:
                wt = [weight_rows(j, m, b) for b in range(NB)]
            blocks = [[w[:, 128 * k:128 * (k + 1)].astype(f32) for k in range(NB)] for w in wt]
            for i, a in enumerate(_lhs_terms(blocks)):
                for p in range(128 // RP):
                    a_v[_term(i, 128, (2 * p + m) * RP // 2, RP // 2)] = _to_words(a[p * RP:(p + 1) * RP])
            for b in range(NB):
                for p in range(128 // RP):
                    ar_v[pl.ds((2 * (p * NB + b) + m) * RP // 2, RP // 2), :] = pltpu.bitcast(
                        wt[b][p * RP:(p + 1) * RP, KS:D], u32)

    def prepare_down(j):
        blocks = [[wd_v[pl.ds(RD * a, RD), chunk_cols(j, b)].astype(f32) for b in range(NB)] for a in range(NB)]
        for i, a in enumerate(_lhs_terms(blocks)):
            ad_v[_term(i, RD // 2, 0, RD // 2)] = _to_words(a)

    def gate_up(t):
        c = pl.ds(128 * t, 128)
        for p in range(128 // RP):
            prod = [None] * TERMS
            for i in TERM_ORDER:
                prod[i] = _dot(_from_words(a_v[_term(i, 128, p * RP, RP)]), _from_words(hb_v[pl.ds(64 * i, 64), c]))
            rest_w = _from_words(ar_v[pl.ds(p * NB * RP, NB * RP), :])
            rest = [_dot(rest_w, _from_words(hr_v[pl.ds(32 * s, 32), c])) for s in range(NB)]
            gu = _assemble(prod)
            gu = [[gu[a][b] + rest[b][2 * a * RP:2 * (a + 1) * RP] for b in range(NB)] for a in range(NB)]
            hidden = [[x[0:RP] * x[RP:2 * RP] for x in row] for row in gu]
            for i, z in enumerate(_rhs_terms(hidden)):
                g_v[_term((t % 2) * TERMS + i, 64, p * RP // 2, RP // 2)] = _to_words(z)

    def down_product(t, i):
        return _dot(_from_words(ad_v[_term(i, RD // 2, 0, RD // 2)]),
                    _from_words(g_v[_term((t % 2) * TERMS + i, 64, 0, 64)]))

    def down(t, first=False):
        for i in TERM_ORDER:
            at = pl.ds(i * RD, RD), pl.ds(128 * t, 128)
            y = down_product(t, i)
            acc_v[at] = y if first else acc_v[at] + y

    def down_and_write(t):
        part = {}
        for g, done in ((1, None), (3, (1, 0)), (2, None), (4, (0, 1)), (0, None), (6, (0, 0)), (5, (1, 1))):
            part[g] = _assemble([acc_v[pl.ds(i * RD, RD), pl.ds(128 * t, 128)] + down_product(t, i)
                                 for i in range(7 * g, 7 * g + 7)])
            if done is None:
                continue
            y = _quadrant(*done, part)
            for s in range(2):
                c = pl.ds(t * FN + 128 * (2 * done[1] + s), 128)
                for a in range(2):
                    r0 = RD * (2 * done[0] + a)
                    out_v[pl.ds(r0, RD), c] = (x1_v[pl.ds(r0, RD), c] + mod(GATE_B, r0, RD) * y[a][s]).astype(bf16)
                rows = pl.ds(done[0] * D // 2, D // 2)
                pltpu.make_async_copy(out_v.at[rows, c], out_hbm.at[rows, c], out_sem).start()

    def glu_chunk(j, last):
        finish = down_and_write if last else down
        down(3)
        gate_up(1)
        prepare_down(j)
        finish(0)
        gate_up(2)
        finish(1)
        gate_up(3)
        if not last:
            prepare_gate_up(j + 1)
        finish(2)
        if last:
            finish(3)
        else:
            gate_up(0)

    got_c = fetch(c_hbm, c_v)
    got_q = fetch(wqkv_hbm, wqkv_v, 0, 640)
    got_mod_a = fetch(wmod_hbm, wmod_v, 0, 2 * D)
    got_x0 = fetch(x_hbm, x_v, 0, TN)
    got_x1 = fetch(x_hbm, x_v, TN, 2 * TN)
    got_k = fetch(wqkv_hbm, wqkv_v, 640, 1152)
    got_v = fetch(wqkv_hbm, wqkv_v, 1152, 3 * D)
    got_x2 = fetch(x_hbm, x_v, 2 * TN, 5 * TN)
    got_x5 = fetch(x_hbm, x_v, 5 * TN, S)
    got_wo = fetch(wo_hbm, wo_v)
    got_mod_b = fetch(wmod_hbm, wmod_v, 2 * D, 6 * D)
    got_glu0 = fetch_glu(0, 1)
    got_glu1 = fetch_glu(1, 2)
    got_glu2 = fetch_glu(2, F // FC)

    acc_v[:, pl.ds(3 * 128, 128)] = jnp.zeros((TERMS * RD, 128), f32)
    wait(got_q)
    prepare_qkv(0)
    wait(got_c, got_mod_a)
    modulation(0, 2 * D)
    wait(got_x0)
    norm_a(0); project(0, 0)
    wait(got_x1, got_k)
    norm_a(1); project(0, 1); prepare_qkv(1)
    wait(got_v)
    project(1, 0); project(1, 1); prepare_qkv(2)
    wait(got_x2)
    project(2, 0); project(2, 1); norm_a(2); norm_a(3)
    project_all(2); attend(0); attend(1)
    project_all(3); norm_a(4); attend(2)
    wait(got_x5, got_wo, got_mod_b, got_glu0, got_glu1)
    prepare_out(); modulation(2 * D, 6 * D); stage_gate_up(0); norm_a(5)
    project_all(4); attention_out(0); attention_out(1); attend(3); norm_b(0); prepare_gate_up()
    attention_out(2); attention_out(3); norm_a(6)
    project_all(5); gate_up(0); attend(4); norm_b(1); norm_a(7)
    project_all(6); gate_up(1); attend(5); prepare_down(0); attention_out(4)
    project_all(7); attend(6); attention_out(5); norm_b(2); down(0, first=True)
    gate_up(2); attend(7); stage_gate_up(1); attention_out(6); attention_out(7); down(1, first=True)
    norm_b(3); gate_up(3); prepare_gate_up(); down(2, first=True); gate_up(0)
    wait(got_glu2)
    lax.fori_loop(1, F // FC - 1, lambda j, carry: glu_chunk(j, False), None)
    glu_chunk(F // FC - 1, True)
    pltpu.make_async_copy(out_v, out_hbm, out_sem).wait()


@jax.jit
def pallas_adaLN_cond__sliding_local_dilated__glu_gated_bilinear__prompt_kernel(
    A_x: jax.Array,
    A_wqkv: jax.Array,
    A_wo: jax.Array,
    B_x: jax.Array,
    B_w_gate: jax.Array,
    B_w_up: jax.Array,
    B_w_down: jax.Array,
    c: jax.Array,
    w_mod: jax.Array,
):
    del B_x
    hbm = pl.BlockSpec(memory_space=pltpu.HBM)
    vmem = pltpu.VMEM
    pairs = (TERMS + 1) // 2
    out = pl.pallas_call(
        _kernel,
        in_specs=[hbm] * 8,
        out_specs=hbm,
        out_shape=jax.ShapeDtypeStruct((D, S), bf16),
        scratch_shapes=[
            vmem((1, D), bf16), vmem((D, 6 * D), bf16), vmem((D, S), bf16),
            vmem((D, 3 * D), bf16), vmem((D, D), bf16), vmem((5, 3 * D, 128), f32),
            vmem((3 * D // 2, 640), u32), vmem((D // 2, 640), u32),
            vmem((6 * D, 128), f32),
            vmem((D // 2, S), u32), vmem((D // 2, S), u32),
            vmem((D // 2, S + 128), u32), vmem((D // 2, S + 128), u32),
            vmem((D // 2, S), u32), vmem((D, S), f32), vmem((16, S), f32),
            vmem((TERMS * 64, S // NB), u32), vmem((NB * 32, S // NB), u32),
            vmem((D, F), bf16), vmem((D, F), bf16), vmem((D, F), bf16),
            vmem((FC, 640), u32),
            vmem((pairs * 128, 256), u32), vmem((FC, D - KS), u32),
            vmem((pairs * RD // 2, 256), u32),
            vmem((TERMS * 64, 256), u32),
            vmem((TERMS * RD, S // NB), f32), vmem((D, S), bf16),
            pltpu.SemaphoreType.DMA((24,)),
        ],
        compiler_params=pltpu.CompilerParams(
            flags={"XLA_TPU_EVENLY_DISTRIBUTE_CRITICAL_NODES": True},
            vmem_limit_bytes=120 * 1024 * 1024),
    )(A_x[0].T, A_wqkv, A_wo, B_w_gate, B_w_up, B_w_down.T, c, w_mod)
    return out.T[None]
```
